```python
import os as _os
_os.environ.setdefault("JAX_PLATFORMS", "cpu")
import jax
import jax.numpy as jnp

def _softmax(x, axis=-1):
    return jax.nn.softmax(x, axis=axis)
def _gelu(x):
    return jax.nn.gelu(x, approximate=True)
def _silu(x):
    return jax.nn.silu(x)
def _sigmoid(x):
    return jax.nn.sigmoid(x)
def _layernorm(x, axis=-1, eps=1e-5):
    m = jnp.mean(x, axis=axis, keepdims=True)
    v = jnp.var(x, axis=axis, keepdims=True)
    return (x - m) / jnp.sqrt(v + eps)
def _scatter_add(tgt, idx, src, axis=0):
    return tgt.at[idx].add(src)
def _segment_sum(src, seg, n):
    return jax.ops.segment_sum(src, seg, n)
class _Rng:
    def __init__(self, key):
        self._k = key
    def _next(self):
        self._k, sub = jax.random.split(self._k)
        return sub
    def normal(self, shape):
        return jax.random.normal(self._next(), shape, dtype=jnp.bfloat16)
    def randint(self, lo, hi, shape):
        return jax.random.randint(self._next(), shape, lo, hi, dtype=jnp.int32)
    def uniform(self, shape, lo=0.0, hi=1.0):
        return jax.random.uniform(self._next(), shape, jnp.bfloat16, lo, hi)
    def permutation(self, n):
        return jax.random.permutation(self._next(), n)


kernel_name = 'recurrent_scan__mha_block__swiglu_ffn__prompt'

def setup_inputs():
    _rng = _Rng(jax.random.key(int.from_bytes(__import__("os").urandom(4), "little")))
    _w = (lambda a: (lambda t: t.astype(jnp.bfloat16) if jnp.issubdtype(t.dtype, jnp.floating) else t)(jnp.asarray(a)))
    def _A_setup():
        B, S, D, H = 1, 2048, 640, 32
        return {
            "x": _w((lambda *s: _rng.normal(s) * 0.05)(B, S, D)),
            "wqkv": _w((lambda *s: _rng.normal(s) * 0.05)(D, 3 * D)),
            "wo": _w((lambda *s: _rng.normal(s) * 0.05)(D, D)),
        }
    _A_in = _A_setup()

    def _B_setup():
        B, S, D, F = 1, 2048, 640, 1728
        return {
            "x": _w((lambda *s: _rng.normal(s) * 0.05)(B, S, D)),
            "w_gate": _w((lambda *s: _rng.normal(s) * 0.05)(D, F)),
            "w_up": _w((lambda *s: _rng.normal(s) * 0.05)(D, F)),
            "w_down": _w((lambda *s: _rng.normal(s) * 0.05)(F, D)),
        }
    _B_in = _B_setup()

    return {
        "A_x": _A_in["x"],
        "A_wqkv": _A_in["wqkv"],
        "A_wo": _A_in["wo"],
        "B_x": _B_in["x"],
        "B_w_gate": _B_in["w_gate"],
        "B_w_up": _B_in["w_up"],
        "B_w_down": _B_in["w_down"],
    }

def reference(A_x, A_wqkv, A_wo, B_x, B_w_gate, B_w_up, B_w_down):
    def _A_ref(x, wqkv, wo):
        B, S, D = x.shape
        H = 32
        Dh = D // H
        qkv = (lambda x, *d: x.transpose(*d))((x @ wqkv).reshape(B, S, 3, H, Dh), 2, 0, 3, 1, 4)
        q, k, v = qkv[0], qkv[1], qkv[2]
        scores = jnp.einsum("bhqd,bhkd->bhqk", q, k) * (Dh ** -0.5)
        p = _softmax(scores, axis=-1)
        o = jnp.einsum("bhqk,bhkd->bhqd", p, v)
        return (lambda x, *d: x.transpose(*d))(o, 0, 2, 1, 3).reshape(B, S, D) @ wo

    def _B_ref(x, w_gate, w_up, w_down):
        g = _silu(x @ w_gate)
        u = x @ w_up
        return (g * u) @ w_down

    x = A_x
    xn = _layernorm(x, axis=-1)
    s = _A_ref(xn, A_wqkv, A_wo)
    g = _silu(_B_ref(xn, B_w_gate, B_w_up, B_w_down))
    return x + s * g
```

```python
import functools
import math

import jax
import jax.numpy as jnp
from jax import lax
import jax.experimental.pallas as pl
import jax.experimental.pallas.tpu as pltpu

S = 2048
D = 640
H = 32
DH = 20
F = 1728
EPS = 1e-5
TA = 512
TC = 512
TQ = 512
KC = 128
NQ = S // TQ
NPAIR = H // 2
NBODY = NPAIR * NQ
QSCALE = (DH ** -0.5) * math.log2(math.e)

_NT = (((1,), (1,)), ((), ()))
_TN = (((0,), (0,)), ((), ()))
f32 = jnp.float32
bf16 = jnp.bfloat16


def _silu(x):
    return x * jax.nn.sigmoid(x)


def _kernel(x_hbm, wqkv_hbm, wo_hbm, wg_hbm, wu_hbm, wd_hbm, out_hbm,
            x_s, wqkv_s, wo_s, wg_s, wu_s, wd_s,
            xn_s, q_s, k_s, wvt_s, vt_s, s0_s, s1_s, m0_s, m1_s, ot_s, out_s,
            xsem, wsem, osem):
    def x_copy(c):
        return pltpu.make_async_copy(
            x_hbm.at[0, pl.ds(c * TA, TA), :], x_s.at[pl.ds(c * TA, TA), :], xsem.at[c])

    w_copies = [
        pltpu.make_async_copy(wqkv_hbm, wqkv_s, wsem.at[0]),
        pltpu.make_async_copy(wg_hbm, wg_s, wsem.at[1]),
        pltpu.make_async_copy(wu_hbm, wu_s, wsem.at[2]),
        pltpu.make_async_copy(wd_hbm, wd_s, wsem.at[3]),
        pltpu.make_async_copy(wo_hbm, wo_s, wsem.at[4]),
    ]
    x_copy(0).start()
    w_copies[0].start()
    for c in range(1, S // TA):
        x_copy(c).start()
    for w in w_copies[1:]:
        w.start()

    lane_a = lax.broadcasted_iota(jnp.int32, (TA, 128), 1)
    sub8 = lax.broadcasted_iota(jnp.int32, (8, TA), 0)
    for c in range(S // TA):
        rows = slice(c * TA, (c + 1) * TA)
        x_copy(c).wait()
        x = x_s[rows, :].astype(f32)
        mu = jnp.mean(x, axis=-1, keepdims=True)
        xc = x - mu
        var = jnp.mean(xc * xc, axis=-1, keepdims=True)
        xn = (xc * lax.rsqrt(var + EPS)).astype(bf16)
        xn_s[rows, :] = xn
        if c == 0:
            w_copies[0].wait()
            wvt_s[...] = wqkv_s[:, 2 * D:3 * D].astype(f32).T.astype(bf16)
        q = jnp.dot(xn, wqkv_s[:, 0:D], preferred_element_type=f32) * QSCALE
        k = jnp.dot(xn, wqkv_s[:, D:2 * D], preferred_element_type=f32)
        for g in range(5):
            q_s[g, rows, :] = q[:, g * 128:(g + 1) * 128].astype(bf16)
            k_s[g, rows, :] = k[:, g * 128:(g + 1) * 128].astype(bf16)
        for g in range(4):
            hi = lane_a >= 64
            q_s[5 + g, rows, :] = jnp.where(
                hi, q[:, g * 128:(g + 1) * 128], q[:, (g + 1) * 128:(g + 2) * 128]).astype(bf16)
            k_s[5 + g, rows, :] = jnp.where(
                hi, k[:, g * 128:(g + 1) * 128], k[:, (g + 1) * 128:(g + 2) * 128]).astype(bf16)
        vt = lax.dot_general(wvt_s[...], xn, _NT, preferred_element_type=f32)
        for p in range(NPAIR):
            b = 40 * p
            mid = vt[b + 16:b + 24, :]
            vt_s[p, 0:16, rows] = vt[b:b + 16, :]
            vt_s[p, 16:24, rows] = jnp.where(sub8 < 4, mid, 1.0)
            vt_s[p, 24:32, rows] = jnp.where(sub8 >= 4, mid, 1.0)
            vt_s[p, 32:48, rows] = vt[b + 24:b + 40, :]

    lane_q = lax.broadcasted_iota(jnp.int32, (TQ, 128), 1)
    sub_q = lax.broadcasted_iota(jnp.int32, (8, TQ), 0)

    def stage(qk, pv):
        if qk is not None:
            h, qi, sq_ref, mq_ref = qk
            col = h * DH
            lo = col % 128
            g = col // 128 + jnp.where(lo > 128 - DH, 5, 0)
            qt = q_s[g, pl.ds(pl.multiple_of(qi * TQ, TQ), TQ), :]
            qm = jnp.where(((lane_q - lo) & 127) < DH, qt, jnp.zeros_like(qt))
            m = None
        if pv is not None:
            pair, par, sp_ref, mp_ref = pv
            mp = mp_ref[0:1, :]
            acc = None
        for c in range(S // KC):
            ks = slice(c * KC, (c + 1) * KC)
            if qk is not None:
                s = lax.dot_general(k_s[g, ks, :], qm, _NT, preferred_element_type=f32)
                sq_ref[ks, :] = s
                mc = jnp.max(s.reshape(KC // 8, 8, TQ), axis=0)
                m = mc if m is None else jnp.maximum(m, mc)
            if pv is not None:
                p = jnp.exp2(sp_ref[ks, :] - mp)
                o = jnp.dot(vt_s[pair, par * 24:(par + 1) * 24, ks], p, preferred_element_type=f32)
                acc = o if acc is None else acc + o
        if qk is not None:
            mq_ref[...] = jnp.broadcast_to(jnp.max(m, axis=0, keepdims=True), (8, TQ))
        if pv is not None:
            l = acc[20:21, :] if par == 0 else acc[0:1, :]
            return acc * (1.0 / l)
        return None

    def store_pair(pair, qi, oa, ob):
        cols = pl.ds(pl.multiple_of(qi * TQ, TQ), TQ)
        mid = jnp.where(sub_q < 4, oa[16:24, :], ob[0:8, :])
        ot_s[pair, :, cols] = jnp.concatenate([oa[0:16, :], mid, ob[8:24, :]], axis=0)

    stage((0, 0, s0_s, m0_s), None)

    def body(j, carry):
        pair = j // NQ
        qi = j % NQ
        jn = j + 1
        oa = stage((2 * pair + 1, qi, s1_s, m1_s), (pair, 0, s0_s, m0_s))
        ob = stage((2 * (jn // NQ), jn % NQ, s0_s, m0_s), (pair, 1, s1_s, m1_s))
        store_pair(pair, qi, oa, ob)
        return carry

    lax.fori_loop(0, NBODY - 1, body, 0)
    oa = stage((H - 1, NQ - 1, s1_s, m1_s), (NPAIR - 1, 0, s0_s, m0_s))
    ob = stage(None, (NPAIR - 1, 1, s1_s, m1_s))
    store_pair(NPAIR - 1, NQ - 1, oa, ob)

    for w in w_copies[1:]:
        w.wait()

    def out_copy(c):
        return pltpu.make_async_copy(
            out_s.at[pl.ds(c * TC, TC), :], out_hbm.at[0, pl.ds(c * TC, TC), :], osem.at[c])

    for c in range(S // TC):
        rows = slice(c * TC, (c + 1) * TC)
        xn = xn_s[rows, :]
        gt = lax.dot_general(xn, wg_s[...], _NT, preferred_element_type=f32)
        up = lax.dot_general(xn, wu_s[...], _NT, preferred_element_type=f32)
        hid = (_silu(gt) * up).astype(bf16)
        ff = jnp.dot(hid, wd_s[...], preferred_element_type=f32)
        ot = ot_s[:, :, rows].reshape(D, TC)
        o = ot.T.astype(bf16)
        sa = jnp.dot(o, wo_s[...], preferred_element_type=f32)
        out_s[rows, :] = (x_s[rows, :].astype(f32) + sa * _silu(ff)).astype(bf16)
        out_copy(c).start()
    for c in range(S // TC):
        out_copy(c).wait()


@jax.jit
def pallas_recurrent_scan__mha_block__swiglu_ffn__prompt_kernel(
    A_x: jax.Array,
    A_wqkv: jax.Array,
    A_wo: jax.Array,
    B_x: jax.Array,
    B_w_gate: jax.Array,
    B_w_up: jax.Array,
    B_w_down: jax.Array,
):
    del B_x
    any_spec = pl.BlockSpec(memory_space=pltpu.HBM)
    return pl.pallas_call(
        _kernel,
        out_shape=jax.ShapeDtypeStruct((1, S, D), bf16),
        in_specs=[any_spec] * 6,
        out_specs=any_spec,
        scratch_shapes=[
            pltpu.VMEM((S, D), bf16),
            pltpu.VMEM((D, 3 * D), bf16),
            pltpu.VMEM((D, D), bf16),
            pltpu.VMEM((F, D), bf16),
            pltpu.VMEM((F, D), bf16),
            pltpu.VMEM((F, D), bf16),
            pltpu.VMEM((S, D), bf16),
            pltpu.VMEM((9, S, 128), bf16),
            pltpu.VMEM((9, S, 128), bf16),
            pltpu.VMEM((D, D), bf16),
            pltpu.VMEM((NPAIR, 48, S), f32),
            pltpu.VMEM((S, TQ), f32),
            pltpu.VMEM((S, TQ), f32),
            pltpu.VMEM((8, TQ), f32),
            pltpu.VMEM((8, TQ), f32),
            pltpu.VMEM((NPAIR, 40, S), f32),
            pltpu.VMEM((S, D), bf16),
            pltpu.SemaphoreType.DMA((S // TA,)),
            pltpu.SemaphoreType.DMA((5,)),
            pltpu.SemaphoreType.DMA((S // TC,)),
        ],
        compiler_params=pltpu.CompilerParams(vmem_limit_bytes=100 * 1024 * 1024),
    )(A_x, A_wqkv, A_wo, B_w_gate.T, B_w_up.T, B_w_down)
```

```python
import math

import jax
import jax.numpy as jnp
from jax import lax
import jax.experimental.pallas as pl
import jax.experimental.pallas.tpu as pltpu

S = 2048
D = 640
H = 32
DH = 20
F = 1728
EPS = 1e-5
TA = 512
TK = 256
XSPLIT = (0, 256, 512, 1024, 2048)
TC = 512
TQ = 512
KC = 128
NT = S // KC
NQ = S // TQ
NCOL = TQ // 128
NPAIR = H // 2
QSCALE = (DH ** -0.5) * math.log2(math.e)
NV = 16
GATES = (0, 5, 10, 15)
L_LO = 2.0 ** -40
L_HI = 2.0 ** 30

_NT = (((1,), (1,)), ((), ()))
f32 = jnp.float32
bf16 = jnp.bfloat16


def _silu(x):
    return x * jax.nn.sigmoid(x)


def _rnd(x):
    return x.astype(bf16).astype(f32)


def _kernel(x_hbm, wqkv_hbm, wo_hbm, wg_hbm, wu_hbm, wd_hbm, out_hbm,
            x_s, wqkv_s, wo_s, wg_s, wu_s, wd_s,
            xn_s, wqt_s, wvt_s, k_s, kp_s, qt_s, vt_s, qn_s, kba_s, kbb_s, ot_s, out_s, sc_s,
            xsem, qsem, wsem, osem):
    def x_copy(i):
        r0, r1 = XSPLIT[i], XSPLIT[i + 1]
        return pltpu.make_async_copy(
            x_hbm.at[0, pl.ds(r0, r1 - r0), :], x_s.at[pl.ds(r0, r1 - r0), :], xsem.at[i])

    def wqkv_copy(j):
        return pltpu.make_async_copy(
            wqkv_hbm.at[:, pl.ds(j * D, D)], wqkv_s.at[:, pl.ds(j * D, D)], qsem.at[j])

    w_copies = [
        pltpu.make_async_copy(wg_hbm, wg_s, wsem.at[0]),
        pltpu.make_async_copy(wu_hbm, wu_s, wsem.at[1]),
        pltpu.make_async_copy(wd_hbm, wd_s, wsem.at[2]),
        pltpu.make_async_copy(wo_hbm, wo_s, wsem.at[3]),
    ]

    lane_a = lax.broadcasted_iota(jnp.int32, (TK // 2, 128), 1)
    sub_a = lax.broadcasted_iota(jnp.int32, (8, TA), 0)
    e_lo = lax.broadcasted_iota(jnp.int32, (H, D), 0) * DH
    e_c = lax.broadcasted_iota(jnp.int32, (H, D), 1)
    et = jnp.where((e_c >= e_lo) & (e_c < e_lo + DH), 1.0, 0.0).astype(f32)
    et16 = et.astype(bf16)
    kmax = [None]

    def layernorm(c):
        rows = slice(c * TK, (c + 1) * TK)
        x = x_s[rows, :].astype(f32)
        mu = jnp.mean(x, axis=-1, keepdims=True)
        xc = x - mu
        var = jnp.mean(xc * xc, axis=-1, keepdims=True)
        xn_s[rows, :] = (xc * lax.rsqrt(var + EPS)).astype(bf16)

    def kproj(c):
        rows = slice(c * TK, (c + 1) * TK)
        k16 = jnp.dot(xn_s[rows, :], wqkv_s[:, D:2 * D], preferred_element_type=f32).astype(bf16)
        k_s[rows, :] = k16
        ku = pltpu.bitcast(k16, jnp.uint32)
        for p in range(NPAIR):
            g, lo = divmod(2 * DH * p, 128)
            tile = ku[:, g * 128:(g + 1) * 128]
            if lo + 2 * DH > 128:
                tile = jnp.where(lane_a >= 64, tile, ku[:, (g + 1) * 128:(g + 2) * 128])
            if lo:
                tile = pltpu.roll(tile, 128 - lo, 1)
            tile = jnp.where(lane_a == 2 * DH, jnp.uint32(0x3F803F80), tile)
            kp_s[p, rows, :] = pltpu.bitcast(tile, bf16).astype(f32)[:, 0:48]

    def knorm(c):
        kf = k_s[c * TK:(c + 1) * TK, :].astype(f32)
        kn = lax.dot_general(et16, (kf * kf).astype(bf16), _NT, preferred_element_type=f32)
        for j in range(TK // 128):
            kj = kn[:, j * 128:(j + 1) * 128]
            kmax[0] = kj if kmax[0] is None else jnp.maximum(kmax[0], kj)

    def vproj(c):
        rows = slice(c * TA, (c + 1) * TA)
        vt = lax.dot_general(wvt_s[...], xn_s[rows, :], _NT, preferred_element_type=f32)
        for p in range(NPAIR):
            b = 40 * p
            mid = vt[b + 16:b + 24, :]
            vt_s[p, 0:16, rows] = vt[b:b + 16, :]
            vt_s[p, 16:24, rows] = jnp.where(sub_a < 4, mid, 1.0)
            vt_s[p, 24:32, rows] = jnp.where(sub_a >= 4, mid, 1.0)
            vt_s[p, 32:48, rows] = vt[b + 24:b + 40, :]

    x_copy(0).start()
    x_copy(1).start()
    wqkv_copy(1).start()
    with jax.named_scope("w_x0"):
        x_copy(0).wait()
    layernorm(0)
    with jax.named_scope("w_x1k"):
        x_copy(1).wait()
        wqkv_copy(1).wait()
    x_copy(2).start()
    x_copy(3).start()
    layernorm(1)
    kproj(0)
    with jax.named_scope("w_x2"):
        x_copy(2).wait()
    wqkv_copy(0).start()
    wqkv_copy(2).start()
    layernorm(2)
    kproj(1)
    layernorm(3)
    kproj(2)
    with jax.named_scope("w_x3"):
        x_copy(3).wait()
    for c in range(3, 6):
        layernorm(c + 1)
        kproj(c)
    with jax.named_scope("w_qv"):
        wqkv_copy(0).wait()
        wqkv_copy(2).wait()
    for w in w_copies:
        w.start()
    layernorm(7)
    wqt_s[...] = wqkv_s[:, 0:D].astype(f32).T.astype(bf16)
    kproj(6)
    wvt_s[...] = wqkv_s[:, 2 * D:3 * D].astype(f32).T.astype(bf16)
    kproj(7)

    qsq = None
    for c in range(S // TA + 1):
        if c < S // TA:
            rows = slice(c * TA, (c + 1) * TA)
            qt = _rnd(lax.dot_general(wqt_s[...], xn_s[rows, :], _NT, preferred_element_type=f32) * QSCALE)
            knorm(2 * c)
            knorm(2 * c + 1)
            for p in range(NPAIR):
                b = 40 * p
                mid = qt[b + 16:b + 24, :]
                qt_s[p, 0:16, rows] = qt[b:b + 16, :]
                qt_s[p, 16:24, rows] = jnp.where(sub_a < 4, mid, 0.0)
                qt_s[p, 24:32, rows] = jnp.where(sub_a >= 4, mid, 0.0)
                qt_s[p, 32:48, rows] = qt[b + 24:b + 40, :]
        else:
            vproj(0)
        if qsq is not None:
            qn_s[:, (c - 1) * TA:c * TA] = jnp.dot(et, qsq, preferred_element_type=f32)
        qsq = qt * qt
    kmax = kmax[0]
    for c in range(1, S // TA):
        vproj(c)

    kmax = jnp.max(kmax, axis=1, keepdims=True)
    qn_s[...] = _rnd(jnp.sqrt(qn_s[...] * kmax) * -1.02)
    sub_s = lax.broadcasted_iota(jnp.int32, (8, S), 0)
    for h in range(H):
        p, par = divmod(h, 2)
        qt_s[p, 48 + 8 * par:56 + 8 * par, :] = jnp.where(sub_s == 0, qn_s[h:h + 1, :], 0.0)

    kbs = (kba_s, kbb_s)

    def sel(never, v8, x):
        n, w = x.shape[0] // 8, x.shape[1]
        return jnp.where(never[None, :, :w], v8[None, :, :w], x.reshape(n, 8, w)).reshape(x.shape)

    def kb_piece(pair, par, t, d0, d1, pin=None):
        src = kp_s[pair, (t + 1) * KC - NV:(t + 1) * KC, :]
        if pin is not None:
            src = sel(pin[0], pin[1], src)
        for d in range(d0, d1):
            ln = DH * par + d
            kbs[par][t, d] = jnp.broadcast_to(src[:, ln:ln + 1], (NV, 128))

    def weights(pair, par, cols, with_bound):
        z16 = jnp.zeros((16, TQ), f32)
        if with_bound:
            mt = qt_s[pair, 48 + 8 * par:56 + 8 * par, cols]
        else:
            mt = jnp.zeros((8, TQ), f32)
        if par == 0:
            return jnp.concatenate([qt_s[pair, 0:24, cols], z16, mt], axis=0)
        return jnp.concatenate([z16, qt_s[pair, 24:48, cols], mt], axis=0)

    def qk(pair, par, qi, t):
        rs = list(range(KC - NV - 8, -1, -8))
        lhs = jnp.concatenate([kp_s[pair, t * KC + r0:t * KC + r0 + 8, :] for r0 in rs], axis=0)
        s = jnp.dot(lhs, weights(pair, par, slice(qi * TQ, (qi + 1) * TQ), True),
                    preferred_element_type=f32)
        e = jnp.exp2(s)
        return s, [e[i * 8:(i + 1) * 8, :] for i in range(len(rs))][::-1]

    def vqk(pair, par, qi, t, never, relv):
        row0 = 28 * par
        css = [slice(qi * TQ + cc * 128, qi * TQ + (cc + 1) * 128) for cc in range(NCOL)]
        cols = [jnp.broadcast_to(qt_s[pair, pl.ds(48 + 8 * par, 1), css[cc]], (NV, 128))
                for cc in range(NCOL)]
        for d in range(DH):
            kb = kbs[par][t, d]
            if relv is not None and d in GATES:
                r = (GATES.index(d) * (relv.shape[0] // 8)) // len(GATES)
                kb = sel(never, relv[r * 8:(r + 1) * 8, 0:128], kb)
            for cc in range(NCOL):
                cols[cc] = cols[cc] + kb * qt_s[pair, pl.ds(row0 + d, 1), css[cc]]
        return jnp.exp2(jnp.concatenate(cols, axis=1))

    for t in range(NT):
        kb_piece(0, 0, t, 0, DH)
        kb_piece(0, 1, t, 0, DH)

    row8 = lax.broadcasted_iota(jnp.int32, (8, 128), 0)
    slots = [(par, t, qi) for par in range(2) for t in range(NT) for qi in range(NQ)]

    def body(pair, bad):
        never = (row8 + pair) < 0
        nxt = jnp.minimum(pair + 1, NPAIR - 1)
        accs = {}

        def do_pv(pend, bad):
            par, t, qi, parts = pend
            o = jnp.dot(vt_s[pair, 24 * par:24 * par + 24, t * KC:(t + 1) * KC],
                        jnp.concatenate(parts, axis=0), preferred_element_type=f32)
            acc = o if t == 0 else o + accs[(par, qi)]
            accs[(par, qi)] = acc
            if t == NT - 1:
                lr = 20 if par == 0 else 0
                l = acc[lr:lr + 1, :]
                ot_s[pair, 24 * par:24 * par + 24, qi * TQ:(qi + 1) * TQ] = acc * (1.0 / l)
                bad = jnp.maximum(bad, jnp.where((l >= L_LO) & (l <= L_HI), 0.0, 1.0))
            return bad

        last = None
        pend = None
        for i, (par, t, qi) in enumerate(slots):
            ev = vqk(pair, par, qi, t, never, last)
            if i >= NQ:
                ppar, pt, _ = slots[i - NQ]
                kb_piece(nxt, ppar, pt, qi * 5, qi * 5 + 5, (never, last[0:8, 0:128]))
            last, parts = qk(pair, par, qi, t)
            parts.append(ev)
            if pend is not None:
                bad = do_pv(pend, bad)
            pend = (par, t, qi, parts)
        kb_piece(nxt, 1, NT - 1, 0, DH)
        return do_pv(pend, bad)

    with jax.named_scope("phaseB"):
        bad = lax.fori_loop(0, NPAIR, body, jnp.zeros((1, TQ), f32))

    @pl.when(jnp.max(bad) > 0.0)
    def _():
        def fb(j, carry):
            pair = j // NQ
            cols = pl.ds(pl.multiple_of((j % NQ) * TQ, TQ), TQ)
            for par in range(2):
                qm = weights(pair, par, cols, False)
                sc_s[...] = jnp.dot(kp_s[pair], qm, preferred_element_type=f32)
                m = jnp.max(sc_s[...], axis=0, keepdims=True)
                p = jnp.exp2(sc_s[...] - m)
                acc = jnp.dot(vt_s[pair, 24 * par:24 * par + 24, :], p, preferred_element_type=f32)
                lr = 20 if par == 0 else 0
                ot_s[pair, 24 * par:24 * par + 24, cols] = acc * (1.0 / acc[lr:lr + 1, :])
            return carry
        lax.fori_loop(0, NPAIR * NQ, fb, 0)

    with jax.named_scope("w_ffn"):
        for w in w_copies:
            w.wait()

    def out_copy(c):
        return pltpu.make_async_copy(
            out_s.at[pl.ds(c * TC, TC), :], out_hbm.at[0, pl.ds(c * TC, TC), :], osem.at[c])

    sub_c = lax.broadcasted_iota(jnp.int32, (8, TC), 0)
    for c in range(S // TC):
        rows = slice(c * TC, (c + 1) * TC)
        xn = xn_s[rows, :]
        gt = lax.dot_general(xn, wg_s[...], _NT, preferred_element_type=f32)
        up = lax.dot_general(xn, wu_s[...], _NT, preferred_element_type=f32)
        hid = (_silu(gt) * up).astype(bf16)
        ff = jnp.dot(hid, wd_s[...], preferred_element_type=f32)
        parts = []
        for p in range(NPAIR):
            parts.append(ot_s[p, 0:16, rows])
            parts.append(jnp.where(sub_c < 4, ot_s[p, 16:24, rows], ot_s[p, 24:32, rows]))
            parts.append(ot_s[p, 32:48, rows])
        o = jnp.concatenate(parts, axis=0).T.astype(bf16)
        sa = jnp.dot(o, wo_s[...], preferred_element_type=f32)
        out_s[rows, :] = (x_s[rows, :].astype(f32) + sa * _silu(ff)).astype(bf16)
        out_copy(c).start()
    with jax.named_scope("w_out"):
        for c in range(S // TC):
            out_copy(c).wait()


@jax.jit
def pallas_recurrent_scan__mha_block__swiglu_ffn__prompt_kernel(
    A_x: jax.Array,
    A_wqkv: jax.Array,
    A_wo: jax.Array,
    B_x: jax.Array,
    B_w_gate: jax.Array,
    B_w_up: jax.Array,
    B_w_down: jax.Array,
):
    del B_x
    hbm = pl.BlockSpec(memory_space=pltpu.HBM)
    return pl.pallas_call(
        _kernel,
        out_shape=jax.ShapeDtypeStruct((1, S, D), bf16),
        in_specs=[hbm] * 6,
        out_specs=hbm,
        scratch_shapes=[
            pltpu.VMEM((S, D), bf16),
            pltpu.VMEM((D, 3 * D), bf16),
            pltpu.VMEM((D, D), bf16),
            pltpu.VMEM((F, D), bf16),
            pltpu.VMEM((F, D), bf16),
            pltpu.VMEM((F, D), bf16),
            pltpu.VMEM((S, D), bf16),
            pltpu.VMEM((D, D), bf16),
            pltpu.VMEM((D, D), bf16),
            pltpu.VMEM((S, D), bf16),
            pltpu.VMEM((NPAIR, S, 48), f32),
            pltpu.VMEM((NPAIR, 64, S), f32),
            pltpu.VMEM((NPAIR, 48, S), f32),
            pltpu.VMEM((H, S), f32),
            pltpu.VMEM((NT, DH, NV, 128), f32),
            pltpu.VMEM((NT, DH, NV, 128), f32),
            pltpu.VMEM((NPAIR, 48, S), f32),
            pltpu.VMEM((S, D), bf16),
            pltpu.VMEM((S, TQ), f32),
            pltpu.SemaphoreType.DMA((4,)),
            pltpu.SemaphoreType.DMA((3,)),
            pltpu.SemaphoreType.DMA((4,)),
            pltpu.SemaphoreType.DMA((S // TC,)),
        ],
        compiler_params=pltpu.CompilerParams(vmem_limit_bytes=110 * 1024 * 1024),
    )(A_x, A_wqkv, A_wo, B_w_gate.T, B_w_up.T, B_w_down)
```

```python
import math

import jax
import jax.numpy as jnp
from jax import lax
import jax.experimental.pallas as pl
import jax.experimental.pallas.tpu as pltpu

S = 2048
D = 640
H = 32
DH = 20
F = 1728
EPS = 1e-5
SH = S // 2
DHALF = D // 2
FH = F // 2
FP = 896
TK = 256
XSPLIT = (0, 256, 512, 1024, 2048)
NB = 256
MQ = 80
LNP = 32
RELSPAN = 3
MF = 144
TNS = (256, 256, 256, 128, 128)
TQ = 512
KC = 128
NT = S // KC
NQ = S // TQ
NCOL = TQ // 128
NPAIR = H // 2
QSCALE = (DH ** -0.5) * math.log2(math.e)
NV = 16
SHIFT = 0
KWA = 32
TOKAT = 3
STAG = (0, 0, 6, 0)
STAGAT = (0,)
ENDPIN = 3
GATES = (0, 5, 10, 15)
L_LO = 2.0 ** -40
L_HI = 2.0 ** 30

_NT = (((1,), (1,)), ((), ()))
f32 = jnp.float32
bf16 = jnp.bfloat16
u32 = jnp.uint32


def _silu(x):
    h = 0.5 * x
    return h * (1.0 + jnp.tanh(h))


def _rnd(x):
    return x.astype(bf16).astype(f32)


def _up(x):
    return x.astype(f32)


def _pk(x):
    return pltpu.bitcast(x.astype(bf16), u32)


def _upk(x):
    return pltpu.bitcast(x, bf16)


def _h2(a, b):
    return slice(a // 2, b // 2)


def _mm(a, b):
    return jnp.dot(a, b, preferred_element_type=f32)


def _nt(a, b):
    return lax.dot_general(a, b, _NT, preferred_element_type=f32)


def _a_sums(a11, a12, a21, a22):
    return a11 + a22, a21 + a22, a11 + a12, a21 - a11, a12 - a22


def _b_sums(b11, b12, b21, b22):
    return b11 + b22, b12 - b22, b21 - b11, b11 + b12, b21 + b22


def _combine(m1, m2, m3, m4, m5, m6, m7):
    return m1 + m4 - m5 + m7, m3 + m5, m2 + m4, m1 - m2 + m3 + m6


def _or_tiles(vals):
    tok = None
    for v in vals:
        for a in range(v.shape[0] // 8):
            for b in range(v.shape[1] // 128):
                t = v[8 * a:8 * a + 8, b * 128:(b + 1) * 128]
                tok = t if tok is None else tok | t
    return tok


def _hold(never, tok, v):
    head = jnp.where(never, tok, v[0:8, 0:128])
    if v.shape[1] > 128:
        head = jnp.concatenate([head, v[0:8, 128:]], axis=1)
    return jnp.concatenate([head, v[8:]], axis=0)


def _kernel(x_hbm, wqkv_hbm, wo_hbm, wg_hbm, wu_hbm, wd_hbm, out_hbm,
            x_s, wqkv_s, wo_s, wg_s, wu_s, wd_s,
            xn_s, xb_s, wt_s, wa_s, k_s, kp_s, qt_s, qw_s, vt_s, kr_s, kba_s, kbb_s, ot_s,
            hb_s, wdt_s, wda_s, out_s, sc_s, pc_s, ev_s,
            sem):
    def x_copy(i):
        r0, r1 = XSPLIT[i], XSPLIT[i + 1]
        return pltpu.make_async_copy(
            x_hbm.at[0, pl.ds(r0, r1 - r0), :], x_s.at[pl.ds(r0, r1 - r0), :], sem.at[i])

    def wqkv_copy(j):
        return pltpu.make_async_copy(
            wqkv_hbm.at[:, pl.ds(j * D, D)], wqkv_s.at[:, pl.ds(j * D, D)], sem.at[1 if j == 1 else 0])

    wd_copy = pltpu.make_async_copy(wd_hbm, wd_s.at[pl.ds(0, F), :], sem.at[1])
    wo_copy = pltpu.make_async_copy(wo_hbm, wo_s, sem.at[1])
    wg_copy = pltpu.make_async_copy(wg_hbm, wg_s, sem.at[1])
    wu_copy = pltpu.make_async_copy(wu_hbm, wu_s, sem.at[1])

    lane_a = lax.broadcasted_iota(jnp.int32, (TK // 2, 128), 1)
    one_lane = jnp.where(lane_a == 0, jnp.uint32(0x3F803F80), jnp.uint32(0))
    sub_b = lax.broadcasted_iota(jnp.int32, (8, NB), 0)
    e_lo = lax.broadcasted_iota(jnp.int32, (H, D), 0) * DH
    e_c = lax.broadcasted_iota(jnp.int32, (H, D), 1)
    et16 = jnp.where((e_c >= e_lo) & (e_c < e_lo + DH), 1.0, 0.0).astype(bf16)
    kmax = [None]
    never_a = [None]

    def sel(never, v8, x):
        n = x.shape[0] // 8
        return jnp.where(never[None], v8[None], x.reshape(n, 8, 128)).reshape(x.shape)

    def gated(v, rel):
        return jnp.concatenate(
            [sel(never_a[0], rel, v[:, g * 128:(g + 1) * 128]) for g in range(v.shape[1] // 128)], axis=1)

    def layernorm(c, rels=None):
        hp = LNP // 2
        for j in range(TK // LNP):
            r0 = c * TK + j * hp
            x = jnp.concatenate([x_s[r0:r0 + hp, :], x_s[r0 + TK // 2:r0 + TK // 2 + hp, :]], axis=0)
            if rels is not None:
                x = _upk(gated(pltpu.bitcast(x, u32), rels[j]))
            x = _up(x)
            mu = jnp.mean(x, axis=-1, keepdims=True)
            xc = x - mu
            var = jnp.mean(xc * xc, axis=-1, keepdims=True)
            if c == 0 and j == 0:
                never_a[0] = jnp.broadcast_to(var[0:8, :], (8, 128)) < -1.0
            xn = xc * lax.rsqrt(var + EPS)
            p0 = c * TK // 2 + j * hp
            lo, hi = xn[0:hp], xn[hp:LNP]
            xn_s[_h2(p0, p0 + hp), :] = _pk(lo)
            xn_s[_h2(SH + p0, SH + p0 + hp), :] = _pk(hi)
            sums = _b_sums(lo[:, 0:256], hi[:, 0:256], lo[:, 256:512], hi[:, 256:512])
            for i in range(5):
                xb_s[i, _h2(p0, p0 + hp), :] = _pk(sums[i])

    def kproj(c):
        lo, hi = _h2(c * TK // 2, (c + 1) * TK // 2), _h2(SH + c * TK // 2, SH + (c + 1) * TK // 2)
        ku = _pk(_mm(_upk(jnp.concatenate([xn_s[lo, :], xn_s[hi, :]], axis=0)), wqkv_s[:, D:2 * D]))
        k_s[lo, :] = ku[0:TK // 4]
        k_s[hi, :] = ku[TK // 4:TK // 2]
        n = TK // LNP
        out = []
        for j in range(n):
            g, i = divmod(j * RELSPAN * 16 // n, 16)
            out.append(ku[8 * i:8 * i + 8, g * 128:(g + 1) * 128])
        return out

    def kpost(c, ku):
        rows = _h2(c * TK, (c + 1) * TK)
        for p in range(NPAIR):
            g, lo = divmod(2 * DH * p, 128)
            tile = ku[:, g * 128:(g + 1) * 128]
            if lo + 2 * DH > 128:
                tile = jnp.where(lane_a >= 64, tile, ku[:, (g + 1) * 128:(g + 2) * 128])
            if lo != 8:
                tile = pltpu.roll(tile, (8 - lo) % 128, 1)
            kp_s[p, rows, :] = jnp.where(lane_a < 8, one_lane, tile)

    def knorm(ku):
        kf = _up(_upk(ku))
        kn = _nt(et16, (kf * kf).astype(bf16))
        for j in range(TK // 128):
            kj = kn[:, j * 128:(j + 1) * 128]
            kmax[0] = kj if kmax[0] is None else jnp.maximum(kmax[0], kj)

    def prep_square(i, w):
        t = _up(w).T
        wt_s[i] = _pk(t)
        sums = _a_sums(t[0:DHALF, 0:256], t[0:DHALF, 256:512], t[DHALF:D, 0:256], t[DHALF:D, 256:512])
        for j in range(5):
            wa_s[i, j] = _pk(sums[j])

    def strassen_x(a, n0, hold=None):
        lo, hi = _h2(n0, n0 + NB), _h2(SH + n0, SH + n0 + NB)
        xe = jnp.concatenate([xn_s[lo, 512:640], xn_s[hi, 512:640]], axis=0)
        if hold is not None:
            xe = _hold(hold[0], hold[1], xe)
        xe = _upk(xe)
        m1 = _nt(a[0], _upk(xb_s[0, lo]))
        m2 = _nt(a[1], _upk(xn_s[lo, 0:256]))
        m3 = _nt(a[2], _upk(xb_s[1, lo]))
        m4 = _nt(a[3], _upk(xb_s[2, lo]))
        m5 = _nt(a[4], _upk(xn_s[hi, 256:512]))
        m6 = _nt(a[5], _upk(xb_s[3, lo]))
        m7 = _nt(a[6], _upk(xb_s[4, lo]))
        e1 = _nt(a[7], xe)
        e2 = _nt(a[8], xe)
        c11, c12, c21, c22 = _combine(m1, m2, m3, m4, m5, m6, m7)
        return c11 + e1[:, 0:NB], c12 + e1[:, NB:], c21 + e2[:, 0:NB], c22 + e2[:, NB:]

    def proj_t(i, n0, r):
        top, bot = _h2(r, r + MQ), _h2(DHALF + r, DHALF + r + MQ)
        a = (_upk(wa_s[i, 0, top]), _upk(wa_s[i, 1, top]), _upk(wt_s[i, top, 0:256]),
             _upk(wt_s[i, bot, 256:512]), _upk(wa_s[i, 2, top]), _upk(wa_s[i, 3, top]),
             _upk(wa_s[i, 4, top]), _upk(wt_s[i, top, 512:640]), _upk(wt_s[i, bot, 512:640]))
        c11, c12, c21, c22 = strassen_x(a, n0)
        lo, hi = slice(n0, n0 + NB), slice(SH + n0, SH + n0 + NB)
        p0 = r // 40
        return ((c11, p0, lo), (c12, p0, hi), (c21, NPAIR // 2 + p0, lo), (c22, NPAIR // 2 + p0, hi))

    def allsum8(v):
        for sh in (4, 2, 1):
            v = v + pltpu.roll(v, sh, 0)
        return v

    def neg_bound(n2, h):
        kr = jnp.concatenate([jnp.broadcast_to(kr_s[pl.ds(h, 1), :], (8, 128))] * (NB // 128), axis=1)
        root = pltpu.bitcast((pltpu.bitcast(n2, jnp.int32) >> 1) + 0x1FC00000, f32)
        return _rnd(root * kr)

    def store_q(qt, p0, cols):
        qt = qt * QSCALE
        z8 = jnp.zeros((8, NB), f32)
        for j in range(MQ // 40):
            p = p0 + j
            t = [qt[40 * j + 8 * i:40 * j + 8 * i + 8, :] for i in range(5)]
            ta, tb = jnp.where(sub_b < 4, t[2], 0.0), jnp.where(sub_b >= 4, t[2], 0.0)
            ma = neg_bound(allsum8(t[0] * t[0] + t[1] * t[1] + ta * ta), 2 * p)
            mb = neg_bound(allsum8(tb * tb + t[3] * t[3] + t[4] * t[4]), 2 * p + 1)
            qt_s[p, :, cols] = jnp.concatenate(t + [ma, mb], axis=0)
            qw_s[2 * p, 0:16, cols] = _pk(jnp.concatenate([ma, t[0], t[1], ta], axis=0))
            qw_s[2 * p + 1, :, cols] = _pk(jnp.concatenate([mb, z8, z8, tb, t[3], t[4]], axis=0))

    def store_v(vt, p0, cols):
        for j in range(MQ // 40):
            b = 40 * j
            mid = vt[b + 16:b + 24, :]
            vt_s[p0 + j, :, cols] = jnp.concatenate(
                [vt[b:b + 16, :], jnp.where(sub_b < 4, mid, 1.0), jnp.where(sub_b >= 4, mid, 1.0),
                 vt[b + 24:b + 40, :]], axis=0)

    x_copy(0).start()
    x_copy(1).start()
    wqkv_copy(1).start()
    x_copy(0).wait()
    layernorm(0)
    x_copy(1).wait()
    wqkv_copy(1).wait()
    x_copy(2).start()
    x_copy(3).start()
    layernorm(1, kproj(0))
    x_copy(2).wait()
    wqkv_copy(2).start()
    wqkv_copy(0).start()
    layernorm(2, kproj(1))
    layernorm(3, kproj(2))
    x_copy(3).wait()
    for c in range(3, 6):
        layernorm(c + 1, kproj(c))
    wqkv_copy(0).wait()
    wqkv_copy(2).wait()
    wg_copy.start()
    wu_copy.start()
    wd_copy.start()
    wo_copy.start()
    prep_square(1, wqkv_s[:, 2 * D:3 * D])
    layernorm(7, kproj(6))
    kproj(7)

    kbs = (kba_s, kbb_s)

    def kb_piece(pair, par, t, d0, d1, pin=None):
        src = kp_s[pair, _h2((t + 1) * KC - NV, (t + 1) * KC), :]
        if pin is not None:
            src = sel(pin[0], pltpu.bitcast(pin[1], u32), src)
        src = _up(_upk(src))
        for d in range(d0, d1):
            ln = 8 + DH * par + d
            kbs[par][t, d] = jnp.broadcast_to(src[:, ln:ln + 1], (NV, 128))

    blocks = [(n0, r) for n0 in range(0, SH, NB) for r in range(0, DHALF, MQ)]
    nh = len(blocks) // 2
    ku = None
    for b, (n0, r) in enumerate(blocks[:nh]):
        outs = proj_t(1, n0, r)
        if ku is not None:
            knorm(ku)
        if b == 0:
            prep_square(0, wqkv_s[:, 0:D])
        for c in range(b * (S // TK) // nh, (b + 1) * (S // TK) // nh):
            ku = gated(k_s[_h2(c * TK, (c + 1) * TK), :], pltpu.bitcast(outs[0][0][0:8, 0:128], u32))
            kpost(c, ku)
        for o in outs:
            store_v(*o)
    for b, (n0, r) in enumerate(blocks):
        outs = proj_t(0, n0, r)
        if b == 0:
            knorm(ku)
            k2 = jnp.max(kmax[0], axis=1, keepdims=True)
            kr_s[...] = jnp.broadcast_to(jnp.sqrt(k2) * -1.02, (H, 128))
        for o in outs:
            store_q(*o)
    for b, (n0, r) in enumerate(blocks[nh:]):
        if b < nh - 1:
            for t in range(b * NT // (nh - 1), (b + 1) * NT // (nh - 1)):
                for par in range(2):
                    kb_piece(0, par, t, 0, DH, (never_a[0], outs[par][0][0:8, 0:128]))
        outs = proj_t(1, n0, r)
        for o in outs:
            store_v(*o)

    def qk(pair, par, qi, t, store, never=None):
        top = KC - NV
        kw = KWA if par == 0 else 48
        gs = [(t, r0) for r0 in range(top - 16 - (SHIFT if t > 0 else 0), -1, -16)]
        if t < NT - 1:
            gs += [(t + 1, r0) for r0 in range(top - 16, top - 16 - SHIFT, -16)]
        lhs = jnp.concatenate(
            [kp_s[pair, _h2(tt * KC + r0, tt * KC + r0 + 16), :] for (tt, r0) in gs], axis=0)
        w = qw_s[2 * pair + par, 0:kw // 2, qi * TQ:(qi + 1) * TQ]
        if never is not None:
            late = qt_s[pair, 0:8, 0:128]
            cols = []
            for cc in range(NCOL):
                for _ in range(STAG[cc]):
                    late = late * 1.5
                wc = w[:, cc * 128:(cc + 1) * 128]
                cols.append(sel(never, pltpu.bitcast(late, u32), wc) if sum(STAG[:cc + 1]) else wc)
            w = jnp.concatenate(cols, axis=1)
        s = _mm(_upk(lhs)[:, 0:kw], _upk(w))
        e = jnp.exp2(s)
        for i, (tt, r0) in enumerate(gs):
            store[(par, qi, tt, r0)] = e[i * 16:(i + 1) * 16, :]
        return s

    def vqk(pair, par, qi, t, never, relv):
        css = [slice(qi * TQ + cc * 128, qi * TQ + (cc + 1) * 128) for cc in range(NCOL)]
        cols = [jnp.concatenate([qt_s[pair, 40 + 8 * par:48 + 8 * par, css[cc]]] * (NV // 8), axis=0)
                for cc in range(NCOL)]
        for d in range(DH):
            kb = kbs[par][t, d]
            if relv is not None and d in GATES:
                r = (GATES.index(d) * (relv.shape[0] // 8)) // len(GATES)
                kb = sel(never, relv[r * 8:(r + 1) * 8, 0:128], kb)
            for cc in range(NCOL):
                cols[cc] = cols[cc] + kb * qt_s[pair, pl.ds(DH * par + d, 1), css[cc]]
        return jnp.exp2(jnp.concatenate(cols, axis=1))

    row8 = lax.broadcasted_iota(jnp.int32, (8, 128), 0)
    slots = [(par, t, qi) for par in range(2) for t in range(NT) for qi in range(NQ)]

    def pv(pair, par, t, qi, p, bad):
        rows, cs = slice(24 * par, 24 * par + 24), slice(qi * TQ, (qi + 1) * TQ)
        acc = _mm(vt_s[pair, rows, t * KC:(t + 1) * KC], p)
        if t > 0:
            acc = acc + ot_s[pair, rows, cs]
        ot_s[pair, rows, cs] = acc
        if t == NT - 1:
            lr = 20 if par == 0 else 0
            l = acc[lr:lr + 1, :]
            bad = jnp.maximum(bad, jnp.where((l >= L_LO) & (l <= L_HI), 0.0, 1.0))
        return bad

    def body(pair, bad):
        never = (row8 + pair) < 0
        nxt = jnp.minimum(pair + 1, NPAIR - 1)
        store = {}

        def p_tile(par, t, qi, ev):
            parts = [store.pop((par, qi, t, r0)) for r0 in range(0, KC - NV, 16)] + [ev]
            return jnp.concatenate(parts, axis=0)

        hist = []
        pend = None
        for i, (par, t, qi) in enumerate(slots):
            ev = vqk(pair, par, qi, t, never, hist[-1]) if hist else ev_s[...]
            if i >= NQ:
                ppar, pt, _ = slots[i - NQ]
                kb_piece(nxt, ppar, pt, qi * 5, qi * 5 + 5, (never, hist[-1][0:8, 0:128]))
            hist.append(qk(pair, par, qi, t, store, never if i in STAGAT else None))
            if pend is None:
                bad = pv(jnp.maximum(pair - 1, 0), *slots[-1], pc_s[...], bad)
            else:
                bad = pv(pair, *pend[:3], p_tile(*pend), bad)
            pend = (par, t, qi, ev)
        kb_piece(nxt, 1, NT - 1, 0, DH, (never, hist[-ENDPIN][0:8, 0:128]))
        pc_s[...] = p_tile(*pend)
        ev_s[...] = vqk(nxt, 0, 0, 0, never, hist[-1])
        return bad

    pc_s[...] = jnp.zeros((KC, TQ), f32)
    ev_s[...] = vqk(0, 0, 0, 0, None, None)
    ot_s[0, 24:48, S - TQ:S] = jnp.ones((24, TQ), f32)
    wg_copy.wait()
    wu_copy.wait()
    wd_copy.wait()
    wo_copy.wait()
    with jax.named_scope("phaseB"):
        bad = lax.fori_loop(0, NPAIR, body, jnp.zeros((1, TQ), f32))
    bad = pv(NPAIR - 1, *slots[-1], pc_s[...], bad)

    never_c = kr_s[0:8, :] > 1.0
    wd_s[F:F + 64, :] = jnp.zeros((64, D), bf16)
    for i in range(7):
        hb_s[i, _h2(FH, FP), :] = jnp.zeros(((FP - FH) // 2, SH), u32)

    def strip_t(w_s, r0, rel):
        v = pltpu.bitcast(w_s[r0:r0 + 128, :], u32)
        relu = pltpu.bitcast(rel, u32)
        v = jnp.concatenate([sel(never_c, relu, v[:, j * 128:(j + 1) * 128]) for j in range(D // 128)], axis=1)
        return _up(_upk(v)).T

    def prep_piece(i, rel):
        if i < FP // 128:
            cs = slice(i * 128, (i + 1) * 128)
            t0, t1 = strip_t(wd_s, i * 128, rel), strip_t(wd_s, FH + i * 128, rel)
            vals = [_pk(v) for v in (t0[0:DHALF], t1[DHALF:D]) + _a_sums(
                t0[0:DHALF], t1[0:DHALF], t0[DHALF:D], t1[DHALF:D])]
            wdt_s[0, :, cs] = vals[0]
            wdt_s[1, :, cs] = vals[1]
            for j in range(5):
                wda_s[j, :, cs] = vals[2 + j]
        elif i < FP // 128 + 2:
            i -= FP // 128
            cs = slice(i * 128, (i + 1) * 128)
            t0, t1 = strip_t(wo_s, i * 128, rel), strip_t(wo_s, 256 + i * 128, rel)
            vals = [_pk(v) for v in (t0, t1) + _a_sums(
                t0[0:DHALF], t1[0:DHALF], t0[DHALF:D], t1[DHALF:D])]
            wt_s[2, :, cs] = vals[0]
            wt_s[2, :, 256 + i * 128:256 + (i + 1) * 128] = vals[1]
            for j in range(5):
                wa_s[2, j, :, cs] = vals[2 + j]
        elif i == FP // 128 + 2:
            vals = [_pk(strip_t(wo_s, 512, rel))]
            wt_s[2, :, 512:640] = vals[0]
        else:
            return None
        return never_c, _or_tiles(vals)

    def ffn_a(w_s, r):
        r1, r2 = slice(r, r + MF), slice(FH + r, FH + r + MF)
        a11, a12, a21, a22 = w_s[r1, 0:256], w_s[r1, 256:512], w_s[r2, 0:256], w_s[r2, 256:512]
        s1, s2, s5, s6, s7 = [v.astype(bf16) for v in _a_sums(_up(a11), _up(a12), _up(a21), _up(a22))]
        return s1, s2, a11, a22, s5, s6, s7, w_s[r1, 512:640], w_s[r2, 512:640]

    blk = 0
    hold = None
    for j in range(FH // MF):
        r = j * MF
        ag, au = ffn_a(wg_s, r), ffn_a(wu_s, r)
        for n0 in range(0, SH, NB):
            g = strassen_x(ag, n0, hold if blk % 2 == 0 else None)
            u = strassen_x(au, n0)
            h11, h12, h21, h22 = [_silu(a) * b for a, b in zip(g, u)]
            t1_, t3, t4, t6, t7 = _b_sums(h11, h12, h21, h22)
            for i, v in enumerate((t1_, h11, t3, t4, h22, t6, t7)):
                hb_s[i, _h2(r, r + MF), n0:n0 + NB] = _pk(v)
            if blk % 2 == 0:
                hold = prep_piece(blk // 2, t7[MF - 8:MF, NB - 128:NB])
            blk += 1

    def out_copy(i):
        return pltpu.make_async_copy(
            out_s.at[pl.ds(i * 128, 128), :], out_hbm.at[0, pl.ds(i * 128, 128), :], sem.at[0])

    def final_block(c0, tn, start_copies, tok=None):
        def ds(a, n):
            return slice(a, a + n) if isinstance(a, int) else pl.ds(pl.multiple_of(a, 128), n)

        sub_n = lax.broadcasted_iota(jnp.int32, (8, tn), 0)

        def o_tile(cs):
            parts = []
            for p in range(NPAIR):
                ra = 1.0 / ot_s[p, 20:21, cs]
                rb = 1.0 / ot_s[p, 24:25, cs]
                parts.append(ot_s[p, 0:16, cs] * ra)
                parts.append(jnp.where(sub_n < 4, ot_s[p, 16:24, cs] * ra, ot_s[p, 24:32, cs] * rb))
                parts.append(ot_s[p, 32:48, cs] * rb)
            return jnp.concatenate(parts, axis=0)

        top, bot = _h2(0, DHALF), _h2(DHALF, D)
        olo, ohi = o_tile(ds(c0, tn)), o_tile(ds(SH + c0, tn))
        b11, b21, b12, b22 = olo[0:256], olo[256:512], ohi[0:256], ohi[256:512]
        t1_, t3, t4, t6, t7 = _b_sums(b11, b12, b21, b22)
        lhs = (wa_s[2, 0], wa_s[2, 1], wt_s[2, top, 0:256], wt_s[2, bot, 256:512],
               wa_s[2, 2], wa_s[2, 3], wa_s[2, 4])
        s11, s12, s21, s22 = _combine(*[
            _mm(_upk(a), b.astype(bf16)) for a, b in zip(lhs, (t1_, b11, t3, t4, b22, t6, t7))])
        e = _mm(_upk(wt_s[2, :, 512:640]),
                jnp.concatenate([olo[512:640], ohi[512:640]], axis=1).astype(bf16))
        lhs = (wda_s[0], wda_s[1], wdt_s[0], wdt_s[1], wda_s[2], wda_s[3], wda_s[4])
        rhs = [hb_s[i, :, ds(c0, tn)] for i in range(7)]
        if tok is not None:
            rhs[TOKAT] = _hold(never_c, tok, rhs[TOKAT])
        f11, f12, f21, f22 = _combine(*[_mm(_upk(a), _upk(b)) for a, b in zip(lhs, rhs)])
        ys = (((jnp.concatenate([s11, s21], axis=0) + e[:, 0:tn])
               * _silu(jnp.concatenate([f11, f21], axis=0))).T,
              ((jnp.concatenate([s12, s22], axis=0) + e[:, tn:])
               * _silu(jnp.concatenate([f12, f22], axis=0))).T)
        done = []
        for j in range(tn // 128):
            for half in range(2):
                r0 = 2 * c0 + (2 * j + half) * 128
                rows = ds(r0, 128)
                o = (_up(x_s[rows, :]) + ys[half][j * 128:(j + 1) * 128]).astype(bf16)
                out_s[rows, :] = o
                if start_copies:
                    out_copy(r0 // 128).start()
                done.append(pltpu.bitcast(o, u32))
        return _or_tiles(done) if start_copies else None

    c0 = 0
    tok = None
    for tn in TNS:
        tok = final_block(c0, tn, True, tok)
        c0 += tn

    @pl.when(jnp.max(bad) > 0.0)
    def _():
        for i in range(S // 128):
            out_copy(i).wait()
        row_q = lax.broadcasted_iota(jnp.int32, (40, TQ), 0)

        def fb(j, carry):
            pair = j // NQ
            cols = pl.ds(pl.multiple_of((j % NQ) * TQ, TQ), TQ)
            for par in range(2):
                mine = (row_q < DH) if par == 0 else (row_q >= DH)
                qm = jnp.concatenate(
                    [jnp.zeros((8, TQ), f32), jnp.where(mine, qt_s[pair, 0:40, cols], 0.0)], axis=0)
                sc_s[...] = _mm(_upk(kp_s[pair])[:, 0:48], qm.astype(bf16))
                m = jnp.max(sc_s[...], axis=0, keepdims=True)
                p = jnp.exp2(sc_s[...] - m)
                ot_s[pair, 24 * par:24 * par + 24, cols] = _mm(vt_s[pair, 24 * par:24 * par + 24, :], p)
            return carry
        lax.fori_loop(0, NPAIR * NQ, fb, 0)

        def redo(c, carry):
            final_block(c * 128, 128, False)
            return carry
        lax.fori_loop(0, SH // 128, redo, 0)
        for i in range(S // 128):
            out_copy(i).start()

    for i in range(S // 128):
        out_copy(i).wait()


@jax.jit
def pallas_recurrent_scan__mha_block__swiglu_ffn__prompt_kernel(
    A_x: jax.Array,
    A_wqkv: jax.Array,
    A_wo: jax.Array,
    B_x: jax.Array,
    B_w_gate: jax.Array,
    B_w_up: jax.Array,
    B_w_down: jax.Array,
):
    del B_x
    hbm = pl.BlockSpec(memory_space=pltpu.HBM)
    return pl.pallas_call(
        _kernel,
        out_shape=jax.ShapeDtypeStruct((1, S, D), bf16),
        in_specs=[hbm] * 6,
        out_specs=hbm,
        scratch_shapes=[
            pltpu.VMEM((S, D), bf16),
            pltpu.VMEM((D, 3 * D), bf16),
            pltpu.VMEM((D, D), bf16),
            pltpu.VMEM((F, D), bf16),
            pltpu.VMEM((F, D), bf16),
            pltpu.VMEM((F + 64, D), bf16),
            pltpu.VMEM((S // 2, D), u32),
            pltpu.VMEM((5, SH // 2, 256), u32),
            pltpu.VMEM((3, D // 2, D), u32),
            pltpu.VMEM((3, 5, DHALF // 2, 256), u32),
            pltpu.VMEM((S // 2, D), u32),
            pltpu.VMEM((NPAIR, S // 2, 128), u32),
            pltpu.VMEM((NPAIR, 56, S), f32),
            pltpu.VMEM((H, 24, S), u32),
            pltpu.VMEM((NPAIR, 48, S), f32),
            pltpu.VMEM((H, 128), f32),
            pltpu.VMEM((NT, DH, NV, 128), f32),
            pltpu.VMEM((NT, DH, NV, 128), f32),
            pltpu.VMEM((NPAIR, 48, S), f32),
            pltpu.VMEM((7, FP // 2, SH), u32),
            pltpu.VMEM((2, DHALF // 2, FP), u32),
            pltpu.VMEM((5, DHALF // 2, FP), u32),
            pltpu.VMEM((S, D), bf16),
            pltpu.VMEM((S, TQ), f32),
            pltpu.VMEM((KC, TQ), f32),
            pltpu.VMEM((NV, TQ), f32),
            pltpu.SemaphoreType.DMA((4,)),
        ],
        compiler_params=pltpu.CompilerParams(vmem_limit_bytes=120 * 1024 * 1024),
    )(A_x, A_wqkv, A_wo, B_w_gate.T, B_w_up.T, B_w_down)
```

```python
import math

import jax
import jax.numpy as jnp
from jax import lax
import jax.experimental.pallas as pl
import jax.experimental.pallas.tpu as pltpu

S = 2048
D = 640
H = 32
DH = 20
F = 1728
EPS = 1e-5
SH = S // 2
DHALF = D // 2
FH = F // 2
FP = 896
TK = 256
LNP = 32
XSPLIT = (0, 256, 512, 1024, 2048)
NB = 256
MQ = 80
MF = 144
TNS = (256, 256, 256, 128, 128)
PREPAT = (0, 1, 4, 5, 8, 9, 12, 13, 16, 17)
TQ = 512
KC = 128
NT = S // KC
NQ = S // TQ
NCOL = TQ // 128
NPAIR = H // 2
QSCALE = (DH ** -0.5) * math.log2(math.e)
NV = 16
GATES = (0, 5, 10, 15)
STAGGER = 6
L_LO = 2.0 ** -40
L_HI = 2.0 ** 30

_NT = (((1,), (1,)), ((), ()))
f32 = jnp.float32
bf16 = jnp.bfloat16
u32 = jnp.uint32


def _silu(x):
    h = 0.5 * x
    return h * (1.0 + jnp.tanh(h))


def _rnd(x):
    return x.astype(bf16).astype(f32)


def _up(x):
    return x.astype(f32)


def _pk(x):
    return pltpu.bitcast(x.astype(bf16), u32)


def _upk(x):
    return pltpu.bitcast(x, bf16)


def _h2(a, b):
    return slice(a // 2, b // 2)


def _mm(a, b):
    return jnp.dot(a, b, preferred_element_type=f32)


def _nt(a, b):
    return lax.dot_general(a, b, _NT, preferred_element_type=f32)


def _a_sums(a11, a12, a21, a22):
    return a11 + a22, a21 + a22, a11 + a12, a21 - a11, a12 - a22


def _b_sums(b11, b12, b21, b22):
    return b11 + b22, b12 - b22, b21 - b11, b11 + b12, b21 + b22


def _combine(m1, m2, m3, m4, m5, m6, m7):
    return m1 + m4 - m5 + m7, m3 + m5, m2 + m4, m1 - m2 + m3 + m6


def _or_tiles(vals):
    tok = None
    for v in vals:
        for a in range(v.shape[0] // 8):
            for b in range(v.shape[1] // 128):
                t = v[8 * a:8 * a + 8, b * 128:(b + 1) * 128]
                tok = t if tok is None else tok | t
    return tok


def _hold(never, tok, v):
    head = jnp.where(never, tok, v[0:8, 0:128])
    if v.shape[1] > 128:
        head = jnp.concatenate([head, v[0:8, 128:]], axis=1)
    return jnp.concatenate([head, v[8:]], axis=0)


def _kernel(x_hbm, wqkv_hbm, wo_hbm, wg_hbm, wu_hbm, wd_hbm, out_hbm,
            x_s, wqkv_s, wo_s, wg_s, wu_s, wd_s,
            xn_s, xb_s, wt_s, wa_s, k_s, kp_s, qt_s, qw_s, vt_s, kr_s, kba_s, kbb_s, ot_s,
            hb_s, wdt_s, wda_s, out_s, sc_s, pc_s, ev_s,
            sem):
    def x_copy(i):
        r0, r1 = XSPLIT[i], XSPLIT[i + 1]
        return pltpu.make_async_copy(
            x_hbm.at[0, pl.ds(r0, r1 - r0), :], x_s.at[pl.ds(r0, r1 - r0), :], sem.at[i])

    def wqkv_copy(j):
        return pltpu.make_async_copy(
            wqkv_hbm.at[:, pl.ds(j * D, D)], wqkv_s.at[:, pl.ds(j * D, D)], sem.at[1 if j == 1 else 0])

    wd_copy = pltpu.make_async_copy(wd_hbm, wd_s.at[pl.ds(0, F), :], sem.at[1])
    wo_copy = pltpu.make_async_copy(wo_hbm, wo_s, sem.at[1])
    wg_copy = pltpu.make_async_copy(wg_hbm, wg_s, sem.at[1])
    wu_copy = pltpu.make_async_copy(wu_hbm, wu_s, sem.at[1])

    lane_a = lax.broadcasted_iota(jnp.int32, (TK // 2, 128), 1)
    one_lane = jnp.where(lane_a == 0, jnp.uint32(0x3F803F80), jnp.uint32(0))
    sub_b = lax.broadcasted_iota(jnp.int32, (8, NB), 0)
    e_lo = lax.broadcasted_iota(jnp.int32, (H, D), 0) * DH
    e_c = lax.broadcasted_iota(jnp.int32, (H, D), 1)
    et16 = jnp.where((e_c >= e_lo) & (e_c < e_lo + DH), 1.0, 0.0).astype(bf16)
    kmax = [None]
    never_a = [None]

    def sel(never, v8, x):
        n = x.shape[0] // 8
        return jnp.where(never[None], v8[None], x.reshape(n, 8, 128)).reshape(x.shape)

    def gated(v, rel):
        return jnp.concatenate(
            [sel(never_a[0], rel, v[:, g * 128:(g + 1) * 128]) for g in range(v.shape[1] // 128)], axis=1)

    def layernorm(c, rels=None):
        hp = LNP // 2
        for j in range(TK // LNP):
            r0 = c * TK + j * hp
            x = jnp.concatenate([x_s[r0:r0 + hp, :], x_s[r0 + TK // 2:r0 + TK // 2 + hp, :]], axis=0)
            if rels is not None:
                x = _upk(gated(pltpu.bitcast(x, u32), rels[j]))
            x = _up(x)
            mu = jnp.mean(x, axis=-1, keepdims=True)
            xc = x - mu
            var = jnp.mean(xc * xc, axis=-1, keepdims=True)
            if c == 0 and j == 0:
                never_a[0] = jnp.broadcast_to(var[0:8, :], (8, 128)) < -1.0
            xn = xc * lax.rsqrt(var + EPS)
            p0 = c * TK // 2 + j * hp
            lo, hi = xn[0:hp], xn[hp:LNP]
            xn_s[_h2(p0, p0 + hp), :] = _pk(lo)
            xn_s[_h2(SH + p0, SH + p0 + hp), :] = _pk(hi)
            sums = _b_sums(lo[:, 0:256], hi[:, 0:256], lo[:, 256:512], hi[:, 256:512])
            for i in range(5):
                xb_s[i, _h2(p0, p0 + hp), :] = _pk(sums[i])

    def kproj(c):
        lo, hi = _h2(c * TK // 2, (c + 1) * TK // 2), _h2(SH + c * TK // 2, SH + (c + 1) * TK // 2)
        ku = _pk(_mm(_upk(jnp.concatenate([xn_s[lo, :], xn_s[hi, :]], axis=0)), wqkv_s[:, D:2 * D]))
        k_s[lo, :] = ku[0:TK // 4]
        k_s[hi, :] = ku[TK // 4:TK // 2]
        n = TK // LNP
        return [ku[8 * (j * 16 // n):8 * (j * 16 // n) + 8, 0:128] for j in range(n)]

    def kpost(c, ku):
        rows = _h2(c * TK, (c + 1) * TK)
        for p in range(NPAIR):
            g, lo = divmod(2 * DH * p, 128)
            tile = ku[:, g * 128:(g + 1) * 128]
            if lo + 2 * DH > 128:
                tile = jnp.where(lane_a >= 64, tile, ku[:, (g + 1) * 128:(g + 2) * 128])
            if lo != 8:
                tile = pltpu.roll(tile, (8 - lo) % 128, 1)
            kp_s[p, rows, :] = jnp.where(lane_a < 8, one_lane, tile)

    def knorm(ku):
        kf = _up(_upk(ku))
        kn = _nt(et16, (kf * kf).astype(bf16))
        for j in range(TK // 128):
            kj = kn[:, j * 128:(j + 1) * 128]
            kmax[0] = kj if kmax[0] is None else jnp.maximum(kmax[0], kj)

    def prep_square(i, w):
        t = _up(w).T
        wt_s[i] = _pk(t)
        sums = _a_sums(t[0:DHALF, 0:256], t[0:DHALF, 256:512], t[DHALF:D, 0:256], t[DHALF:D, 256:512])
        for j in range(5):
            wa_s[i, j] = _pk(sums[j])

    def strassen_x(a, n0, hold=None):
        lo, hi = _h2(n0, n0 + NB), _h2(SH + n0, SH + n0 + NB)
        xe = jnp.concatenate([xn_s[lo, 512:640], xn_s[hi, 512:640]], axis=0)
        if hold is not None:
            xe = _hold(hold[0], hold[1], xe)
        xe = _upk(xe)
        m1 = _nt(a[0], _upk(xb_s[0, lo]))
        m2 = _nt(a[1], _upk(xn_s[lo, 0:256]))
        m3 = _nt(a[2], _upk(xb_s[1, lo]))
        m4 = _nt(a[3], _upk(xb_s[2, lo]))
        m5 = _nt(a[4], _upk(xn_s[hi, 256:512]))
        m6 = _nt(a[5], _upk(xb_s[3, lo]))
        m7 = _nt(a[6], _upk(xb_s[4, lo]))
        e1 = _nt(a[7], xe)
        e2 = _nt(a[8], xe)
        c11, c12, c21, c22 = _combine(m1, m2, m3, m4, m5, m6, m7)
        return c11 + e1[:, 0:NB], c12 + e1[:, NB:], c21 + e2[:, 0:NB], c22 + e2[:, NB:]

    def proj_t(i, n0, r):
        top, bot = _h2(r, r + MQ), _h2(DHALF + r, DHALF + r + MQ)
        a = (_upk(wa_s[i, 0, top]), _upk(wa_s[i, 1, top]), _upk(wt_s[i, top, 0:256]),
             _upk(wt_s[i, bot, 256:512]), _upk(wa_s[i, 2, top]), _upk(wa_s[i, 3, top]),
             _upk(wa_s[i, 4, top]), _upk(wt_s[i, top, 512:640]), _upk(wt_s[i, bot, 512:640]))
        c11, c12, c21, c22 = strassen_x(a, n0)
        lo, hi = slice(n0, n0 + NB), slice(SH + n0, SH + n0 + NB)
        p0 = r // 40
        return ((c11, p0, lo), (c12, p0, hi), (c21, NPAIR // 2 + p0, lo), (c22, NPAIR // 2 + p0, hi))

    def allsum8(v):
        for sh in (4, 2, 1):
            v = v + pltpu.roll(v, sh, 0)
        return v

    def neg_bound(n2, h):
        kr = jnp.concatenate([jnp.broadcast_to(kr_s[pl.ds(h, 1), :], (8, 128))] * (NB // 128), axis=1)
        root = pltpu.bitcast((pltpu.bitcast(n2, jnp.int32) >> 1) + 0x1FC00000, f32)
        return _rnd(root * kr)

    def store_q(qt, p0, cols):
        qt = qt * QSCALE
        z8 = jnp.zeros((8, NB), f32)
        for j in range(MQ // 40):
            p = p0 + j
            t = [qt[40 * j + 8 * i:40 * j + 8 * i + 8, :] for i in range(5)]
            ta, tb = jnp.where(sub_b < 4, t[2], 0.0), jnp.where(sub_b >= 4, t[2], 0.0)
            ma = neg_bound(allsum8(t[0] * t[0] + t[1] * t[1] + ta * ta), 2 * p)
            mb = neg_bound(allsum8(tb * tb + t[3] * t[3] + t[4] * t[4]), 2 * p + 1)
            qt_s[p, :, cols] = jnp.concatenate(t + [ma, mb], axis=0)
            qw_s[2 * p, 0:16, cols] = _pk(jnp.concatenate([ma, t[0], t[1], ta], axis=0))
            qw_s[2 * p + 1, :, cols] = _pk(jnp.concatenate([mb, z8, z8, tb, t[3], t[4]], axis=0))

    def store_v(vt, p0, cols):
        for j in range(MQ // 40):
            b = 40 * j
            mid = vt[b + 16:b + 24, :]
            vt_s[p0 + j, :, cols] = jnp.concatenate(
                [vt[b:b + 16, :], jnp.where(sub_b < 4, mid, 1.0), jnp.where(sub_b >= 4, mid, 1.0),
                 vt[b + 24:b + 40, :]], axis=0)

    x_copy(0).start()
    x_copy(1).start()
    wqkv_copy(1).start()
    x_copy(0).wait()
    layernorm(0)
    x_copy(1).wait()
    wqkv_copy(1).wait()
    x_copy(2).start()
    x_copy(3).start()
    layernorm(1, kproj(0))
    x_copy(2).wait()
    wqkv_copy(2).start()
    wqkv_copy(0).start()
    layernorm(2, kproj(1))
    layernorm(3, kproj(2))
    x_copy(3).wait()
    for c in range(3, 6):
        layernorm(c + 1, kproj(c))
    wqkv_copy(0).wait()
    wqkv_copy(2).wait()
    wg_copy.start()
    wu_copy.start()
    wd_copy.start()
    wo_copy.start()
    prep_square(1, wqkv_s[:, 2 * D:3 * D])
    layernorm(7, kproj(6))
    kproj(7)

    kbs = (kba_s, kbb_s)

    def kb_piece(pair, par, t, d0, d1, pin=None):
        src = kp_s[pair, _h2((t + 1) * KC - NV, (t + 1) * KC), :]
        if pin is not None:
            src = sel(pin[0], pltpu.bitcast(pin[1], u32), src)
        src = _up(_upk(src))
        for d in range(d0, d1):
            ln = 8 + DH * par + d
            kbs[par][t, d] = jnp.broadcast_to(src[:, ln:ln + 1], (NV, 128))

    blocks = [(n0, r) for n0 in range(0, SH, NB) for r in range(0, DHALF, MQ)]
    nh = len(blocks) // 2
    ku = None
    for b, (n0, r) in enumerate(blocks[:nh]):
        outs = proj_t(1, n0, r)
        if ku is not None:
            knorm(ku)
        if b == 0:
            prep_square(0, wqkv_s[:, 0:D])
        for c in range(b * (S // TK) // nh, (b + 1) * (S // TK) // nh):
            ku = gated(k_s[_h2(c * TK, (c + 1) * TK), :], pltpu.bitcast(outs[0][0][0:8, 0:128], u32))
            kpost(c, ku)
        for o in outs:
            store_v(*o)
    for b, (n0, r) in enumerate(blocks):
        outs = proj_t(0, n0, r)
        if b == 0:
            knorm(ku)
            k2 = jnp.max(kmax[0], axis=1, keepdims=True)
            kr_s[...] = jnp.broadcast_to(jnp.sqrt(k2) * -1.02, (H, 128))
        for o in outs:
            store_q(*o)
    for b, (n0, r) in enumerate(blocks[nh:]):
        if b < nh - 1:
            for t in range(b * NT // (nh - 1), (b + 1) * NT // (nh - 1)):
                for par in range(2):
                    kb_piece(0, par, t, 0, DH, (never_a[0], outs[par][0][0:8, 0:128]))
        outs = proj_t(1, n0, r)
        for o in outs:
            store_v(*o)

    def qk(pair, par, qi, t, never=None):
        kw = 32 if par == 0 else 48
        rs = list(range(KC - NV - 16, -1, -16))
        lhs = jnp.concatenate([kp_s[pair, _h2(t * KC + r0, t * KC + r0 + 16), :] for r0 in rs], axis=0)
        w = qw_s[2 * pair + par, 0:kw // 2, qi * TQ:(qi + 1) * TQ]
        if never is not None:
            late = qt_s[pair, 0:8, 0:128]
            for _ in range(STAGGER):
                late = late * 1.5
            late = pltpu.bitcast(late, u32)
            w = jnp.concatenate(
                [w[:, 0:128], w[:, 128:256], sel(never, late, w[:, 256:384]), sel(never, late, w[:, 384:512])],
                axis=1)
        s = _mm(_upk(lhs)[:, 0:kw], _upk(w))
        e = jnp.exp2(s)
        return s, [e[i * 16:(i + 1) * 16, :] for i in range(len(rs))][::-1]

    def vqk(pair, par, qi, t, never, relv):
        css = [slice(qi * TQ + cc * 128, qi * TQ + (cc + 1) * 128) for cc in range(NCOL)]
        cols = [jnp.concatenate([qt_s[pair, 40 + 8 * par:48 + 8 * par, css[cc]]] * (NV // 8), axis=0)
                for cc in range(NCOL)]
        for d in range(DH):
            kb = kbs[par][t, d]
            if relv is not None and d in GATES:
                r = (GATES.index(d) * (relv.shape[0] // 8)) // len(GATES)
                kb = sel(never, relv[r * 8:(r + 1) * 8, 0:128], kb)
            for cc in range(NCOL):
                cols[cc] = cols[cc] + kb * qt_s[pair, pl.ds(DH * par + d, 1), css[cc]]
        return jnp.exp2(jnp.concatenate(cols, axis=1))

    row8 = lax.broadcasted_iota(jnp.int32, (8, 128), 0)
    slots = [(par, t, qi) for par in range(2) for t in range(NT) for qi in range(NQ)]

    def pv(pair, par, t, qi, p, bad):
        rows, cs = slice(24 * par, 24 * par + 24), slice(qi * TQ, (qi + 1) * TQ)
        acc = _mm(vt_s[pair, rows, t * KC:(t + 1) * KC], p)
        if t > 0:
            acc = acc + ot_s[pair, rows, cs]
        ot_s[pair, rows, cs] = acc
        if t == NT - 1:
            lr = 20 if par == 0 else 0
            l = acc[lr:lr + 1, :]
            bad = jnp.maximum(bad, jnp.where((l >= L_LO) & (l <= L_HI), 0.0, 1.0))
        return bad

    def body(pair, bad):
        never = (row8 + pair) < 0
        nxt = jnp.minimum(pair + 1, NPAIR - 1)
        hist = []
        pend = None
        for i, (par, t, qi) in enumerate(slots):
            ev = vqk(pair, par, qi, t, never, hist[-1]) if hist else ev_s[...]
            if i >= NQ:
                ppar, pt, _ = slots[i - NQ]
                kb_piece(nxt, ppar, pt, qi * 5, qi * 5 + 5, (never, hist[-1][0:8, 0:128]))
            s, parts = qk(pair, par, qi, t, never if i == 0 else None)
            hist.append(s)
            if pend is None:
                bad = pv(jnp.maximum(pair - 1, 0), *slots[-1], pc_s[...], bad)
            else:
                bad = pv(pair, *pend[:3], jnp.concatenate(pend[3], axis=0), bad)
            pend = (par, t, qi, parts + [ev])
        kb_piece(nxt, 1, NT - 1, 0, DH, (never, hist[-3][0:8, 0:128]))
        pc_s[...] = jnp.concatenate(pend[3], axis=0)
        ev_s[...] = vqk(nxt, 0, 0, 0, never, hist[-1])
        return bad

    pc_s[...] = jnp.zeros((KC, TQ), f32)
    ev_s[...] = vqk(0, 0, 0, 0, None, None)
    ot_s[0, 24:48, S - TQ:S] = jnp.ones((24, TQ), f32)
    wg_copy.wait()
    wu_copy.wait()
    wd_copy.wait()
    wo_copy.wait()
    bad = lax.fori_loop(0, NPAIR, body, jnp.zeros((1, TQ), f32))
    bad = pv(NPAIR - 1, *slots[-1], pc_s[...], bad)

    never_c = kr_s[0:8, :] > 1.0
    wd_s[F:F + 64, :] = jnp.zeros((64, D), bf16)
    for i in range(7):
        hb_s[i, _h2(FH, FP), :] = jnp.zeros(((FP - FH) // 2, SH), u32)

    def strip_t(w_s, r0, rel):
        v = pltpu.bitcast(w_s[r0:r0 + 128, :], u32)
        relu = pltpu.bitcast(rel, u32)
        v = jnp.concatenate([sel(never_c, relu, v[:, j * 128:(j + 1) * 128]) for j in range(D // 128)], axis=1)
        return _up(_upk(v)).T

    def prep_piece(i, rel):
        if i < FP // 128:
            cs = slice(i * 128, (i + 1) * 128)
            t0, t1 = strip_t(wd_s, i * 128, rel), strip_t(wd_s, FH + i * 128, rel)
            vals = [_pk(v) for v in (t0[0:DHALF], t1[DHALF:D]) + _a_sums(
                t0[0:DHALF], t1[0:DHALF], t0[DHALF:D], t1[DHALF:D])]
            wdt_s[0, :, cs] = vals[0]
            wdt_s[1, :, cs] = vals[1]
            for j in range(5):
                wda_s[j, :, cs] = vals[2 + j]
        elif i < FP // 128 + 2:
            i -= FP // 128
            cs = slice(i * 128, (i + 1) * 128)
            t0, t1 = strip_t(wo_s, i * 128, rel), strip_t(wo_s, 256 + i * 128, rel)
            vals = [_pk(v) for v in (t0, t1) + _a_sums(
                t0[0:DHALF], t1[0:DHALF], t0[DHALF:D], t1[DHALF:D])]
            wt_s[2, :, cs] = vals[0]
            wt_s[2, :, 256 + i * 128:256 + (i + 1) * 128] = vals[1]
            for j in range(5):
                wa_s[2, j, :, cs] = vals[2 + j]
        else:
            vals = [_pk(strip_t(wo_s, 512, rel))]
            wt_s[2, :, 512:640] = vals[0]
        return never_c, _or_tiles(vals)

    def ffn_a(w_s, r):
        r1, r2 = slice(r, r + MF), slice(FH + r, FH + r + MF)
        a11, a12, a21, a22 = w_s[r1, 0:256], w_s[r1, 256:512], w_s[r2, 0:256], w_s[r2, 256:512]
        s1, s2, s5, s6, s7 = [v.astype(bf16) for v in _a_sums(_up(a11), _up(a12), _up(a21), _up(a22))]
        return s1, s2, a11, a22, s5, s6, s7, w_s[r1, 512:640], w_s[r2, 512:640]

    blk = 0
    holds = {}
    for j in range(FH // MF):
        r = j * MF
        ag, au = ffn_a(wg_s, r), ffn_a(wu_s, r)
        for n0 in range(0, SH, NB):
            g = strassen_x(ag, n0, holds.pop(blk, None))
            u = strassen_x(au, n0)
            h11, h12, h21, h22 = [_silu(a) * b for a, b in zip(g, u)]
            t1_, t3, t4, t6, t7 = _b_sums(h11, h12, h21, h22)
            for i, v in enumerate((t1_, h11, t3, t4, h22, t6, t7)):
                hb_s[i, _h2(r, r + MF), n0:n0 + NB] = _pk(v)
            if blk in PREPAT:
                holds[blk + 2] = prep_piece(PREPAT.index(blk), t7[MF - 8:MF, NB - 128:NB])
            blk += 1

    def out_copy(i):
        return pltpu.make_async_copy(
            out_s.at[pl.ds(i * 128, 128), :], out_hbm.at[0, pl.ds(i * 128, 128), :], sem.at[0])

    def final_block(c0, tn, start_copies, tok=None):
        def ds(a, n):
            return slice(a, a + n) if isinstance(a, int) else pl.ds(pl.multiple_of(a, 128), n)

        sub_n = lax.broadcasted_iota(jnp.int32, (8, tn), 0)

        def o_tile(cs):
            parts = []
            for p in range(NPAIR):
                ra = 1.0 / ot_s[p, 20:21, cs]
                rb = 1.0 / ot_s[p, 24:25, cs]
                parts.append(ot_s[p, 0:16, cs] * ra)
                parts.append(jnp.where(sub_n < 4, ot_s[p, 16:24, cs] * ra, ot_s[p, 24:32, cs] * rb))
                parts.append(ot_s[p, 32:48, cs] * rb)
            return jnp.concatenate(parts, axis=0)

        top, bot = _h2(0, DHALF), _h2(DHALF, D)
        olo, ohi = o_tile(ds(c0, tn)), o_tile(ds(SH + c0, tn))
        b11, b21, b12, b22 = olo[0:256], olo[256:512], ohi[0:256], ohi[256:512]
        t1_, t3, t4, t6, t7 = _b_sums(b11, b12, b21, b22)
        lhs = (wa_s[2, 0], wa_s[2, 1], wt_s[2, top, 0:256], wt_s[2, bot, 256:512],
               wa_s[2, 2], wa_s[2, 3], wa_s[2, 4])
        s11, s12, s21, s22 = _combine(*[
            _mm(_upk(a), b.astype(bf16)) for a, b in zip(lhs, (t1_, b11, t3, t4, b22, t6, t7))])
        e = _mm(_upk(wt_s[2, :, 512:640]),
                jnp.concatenate([olo[512:640], ohi[512:640]], axis=1).astype(bf16))
        lhs = (wda_s[0], wda_s[1], wdt_s[0], wdt_s[1], wda_s[2], wda_s[3], wda_s[4])
        rhs = [hb_s[i, :, ds(c0, tn)] for i in range(7)]
        if tok is not None:
            rhs[3] = _hold(never_c, tok, rhs[3])
        f11, f12, f21, f22 = _combine(*[_mm(_upk(a), _upk(b)) for a, b in zip(lhs, rhs)])
        ys = (((jnp.concatenate([s11, s21], axis=0) + e[:, 0:tn])
               * _silu(jnp.concatenate([f11, f21], axis=0))).T,
              ((jnp.concatenate([s12, s22], axis=0) + e[:, tn:])
               * _silu(jnp.concatenate([f12, f22], axis=0))).T)
        done = []
        for j in range(tn // 128):
            for half in range(2):
                r0 = 2 * c0 + (2 * j + half) * 128
                rows = ds(r0, 128)
                o = (_up(x_s[rows, :]) + ys[half][j * 128:(j + 1) * 128]).astype(bf16)
                out_s[rows, :] = o
                if start_copies:
                    out_copy(r0 // 128).start()
                done.append(pltpu.bitcast(o, u32))
        return _or_tiles(done) if start_copies else None

    c0 = 0
    tok = None
    for tn in TNS:
        tok = final_block(c0, tn, True, tok)
        c0 += tn

    @pl.when(jnp.max(bad) > 0.0)
    def _():
        for i in range(S // 128):
            out_copy(i).wait()
        row_q = lax.broadcasted_iota(jnp.int32, (40, TQ), 0)

        def fb(j, carry):
            pair = j // NQ
            cols = pl.ds(pl.multiple_of((j % NQ) * TQ, TQ), TQ)
            for par in range(2):
                mine = (row_q < DH) if par == 0 else (row_q >= DH)
                qm = jnp.concatenate(
                    [jnp.zeros((8, TQ), f32), jnp.where(mine, qt_s[pair, 0:40, cols], 0.0)], axis=0)
                sc_s[...] = _mm(_upk(kp_s[pair])[:, 0:48], qm.astype(bf16))
                m = jnp.max(sc_s[...], axis=0, keepdims=True)
                p = jnp.exp2(sc_s[...] - m)
                ot_s[pair, 24 * par:24 * par + 24, cols] = _mm(vt_s[pair, 24 * par:24 * par + 24, :], p)
            return carry
        lax.fori_loop(0, NPAIR * NQ, fb, 0)

        def redo(c, carry):
            final_block(c * 128, 128, False)
            return carry
        lax.fori_loop(0, SH // 128, redo, 0)
        for i in range(S // 128):
            out_copy(i).start()

    for i in range(S // 128):
        out_copy(i).wait()


@jax.jit
def pallas_recurrent_scan__mha_block__swiglu_ffn__prompt_kernel(
    A_x: jax.Array,
    A_wqkv: jax.Array,
    A_wo: jax.Array,
    B_x: jax.Array,
    B_w_gate: jax.Array,
    B_w_up: jax.Array,
    B_w_down: jax.Array,
):
    del B_x
    hbm = pl.BlockSpec(memory_space=pltpu.HBM)
    return pl.pallas_call(
        _kernel,
        out_shape=jax.ShapeDtypeStruct((1, S, D), bf16),
        in_specs=[hbm] * 6,
        out_specs=hbm,
        scratch_shapes=[
            pltpu.VMEM((S, D), bf16),
            pltpu.VMEM((D, 3 * D), bf16),
            pltpu.VMEM((D, D), bf16),
            pltpu.VMEM((F, D), bf16),
            pltpu.VMEM((F, D), bf16),
            pltpu.VMEM((F + 64, D), bf16),
            pltpu.VMEM((S // 2, D), u32),
            pltpu.VMEM((5, SH // 2, 256), u32),
            pltpu.VMEM((3, D // 2, D), u32),
            pltpu.VMEM((3, 5, DHALF // 2, 256), u32),
            pltpu.VMEM((S // 2, D), u32),
            pltpu.VMEM((NPAIR, S // 2, 128), u32),
            pltpu.VMEM((NPAIR, 56, S), f32),
            pltpu.VMEM((H, 24, S), u32),
            pltpu.VMEM((NPAIR, 48, S), f32),
            pltpu.VMEM((H, 128), f32),
            pltpu.VMEM((NT, DH, NV, 128), f32),
            pltpu.VMEM((NT, DH, NV, 128), f32),
            pltpu.VMEM((NPAIR, 48, S), f32),
            pltpu.VMEM((7, FP // 2, SH), u32),
            pltpu.VMEM((2, DHALF // 2, FP), u32),
            pltpu.VMEM((5, DHALF // 2, FP), u32),
            pltpu.VMEM((S, D), bf16),
            pltpu.VMEM((S, TQ), f32),
            pltpu.VMEM((KC, TQ), f32),
            pltpu.VMEM((NV, TQ), f32),
            pltpu.SemaphoreType.DMA((4,)),
        ],
        compiler_params=pltpu.CompilerParams(vmem_limit_bytes=120 * 1024 * 1024),
    )(A_x, A_wqkv, A_wo, B_w_gate.T, B_w_up.T, B_w_down)
```

```python
import math

import jax
import jax.numpy as jnp
from jax import lax
import jax.experimental.pallas as pl
import jax.experimental.pallas.tpu as pltpu

S = 2048
D = 640
H = 32
DH = 20
F = 1728
EPS = 1e-5
SH = S // 2
DHALF = D // 2
FH = F // 2
FP = 896
TK = 256
LNP = 32
XSPLIT = (0, 256, 512, 1024, 2048)
NB = 256
MQ = 80
MF = 144
TNS = (256, 256, 256, 128, 128)
PREPAT = (0, 1, 4, 5, 8, 9, 12, 13, 16, 17)
TQ = 512
KC = 128
NT = S // KC
NQ = S // TQ
NCOL = TQ // 128
NPAIR = H // 2
QSCALE = (DH ** -0.5) * math.log2(math.e)
NV = 16
GATES = (0, 5, 10, 15)
STAGGER = 6
L_LO = 2.0 ** -40
L_HI = 2.0 ** 30

_NT = (((1,), (1,)), ((), ()))
f32 = jnp.float32
bf16 = jnp.bfloat16
u32 = jnp.uint32
_ALL = slice(None)


def _silu(x):
    h = 0.5 * x
    return h * (1.0 + jnp.tanh(h))


def _rnd(x):
    return x.astype(bf16).astype(f32)


def _up(x):
    return x.astype(f32)


def _pk(x):
    return pltpu.bitcast(x.astype(bf16), u32)


def _put(ref, lead, rows, cols, x):
    idx = tuple(slice(i, i + 1) for i in lead) + (rows, cols)
    ref[idx] = _pk(x.reshape((1,) * len(lead) + x.shape))


def _bits(x):
    return pltpu.bitcast(x, u32)


def _upk(x):
    return pltpu.bitcast(x, bf16)


def _h2(a, b):
    return slice(a // 2, b // 2)


def _mm(a, b):
    return jnp.dot(a, b, preferred_element_type=f32)


def _nt(a, b):
    return lax.dot_general(a, b, _NT, preferred_element_type=f32)


def _a_sums(a11, a12, a21, a22):
    return a11 + a22, a21 + a22, a11 + a12, a21 - a11, a12 - a22


def _b_sums(b11, b12, b21, b22):
    return b11 + b22, b12 - b22, b21 - b11, b11 + b12, b21 + b22


def _combine(m1, m2, m3, m4, m5, m6, m7):
    return m1 + m4 - m5 + m7, m3 + m5, m2 + m4, m1 - m2 + m3 + m6


def _or_tiles(vals):
    tok = None
    for v in vals:
        for a in range(v.shape[0] // 8):
            for b in range(v.shape[1] // 128):
                t = v[8 * a:8 * a + 8, b * 128:(b + 1) * 128]
                tok = t if tok is None else tok | t
    return tok


def _hold(never, tok, v):
    head = jnp.where(never, tok, v[0:8, 0:128])
    if v.shape[1] > 128:
        head = jnp.concatenate([head, v[0:8, 128:]], axis=1)
    return jnp.concatenate([head, v[8:]], axis=0)


def _kernel(x_hbm, wqkv_hbm, wo_hbm, wg_hbm, wu_hbm, wd_hbm, out_hbm,
            x_s, wqkv_s, wo_s, wg_s, wu_s, wd_s,
            xn_s, xb_s, wt_s, wa_s, k_s, kp_s, qt_s, qw_s, vt_s, kr_s, kba_s, kbb_s, ot_s,
            hb_s, wdt_s, wda_s, out_s, sc_s, pc_s, ev_s,
            sem):
    def x_copy(i):
        r0, r1 = XSPLIT[i], XSPLIT[i + 1]
        return pltpu.make_async_copy(
            x_hbm.at[0, pl.ds(r0, r1 - r0), :], x_s.at[pl.ds(r0, r1 - r0), :], sem.at[i])

    def wqkv_copy(j):
        return pltpu.make_async_copy(
            wqkv_hbm.at[:, pl.ds(j * D, D)], wqkv_s.at[:, pl.ds(j * D, D)], sem.at[1 if j == 1 else 0])

    wd_copy = pltpu.make_async_copy(wd_hbm, wd_s.at[pl.ds(0, F), :], sem.at[1])
    wo_copy = pltpu.make_async_copy(wo_hbm, wo_s, sem.at[1])
    wg_copy = pltpu.make_async_copy(wg_hbm, wg_s, sem.at[1])
    wu_copy = pltpu.make_async_copy(wu_hbm, wu_s, sem.at[1])

    lane_a = lax.broadcasted_iota(jnp.int32, (TK // 2, 128), 1)
    one_lane = jnp.where(lane_a == 0, jnp.uint32(0x3F803F80), jnp.uint32(0))
    sub_b = lax.broadcasted_iota(jnp.int32, (8, NB), 0)
    e_lo = lax.broadcasted_iota(jnp.int32, (H, D), 0) * DH
    e_c = lax.broadcasted_iota(jnp.int32, (H, D), 1)
    et16 = jnp.where((e_c >= e_lo) & (e_c < e_lo + DH), 1.0, 0.0).astype(bf16)
    kmax = [None]
    never_a = [None]

    def sel(never, v8, x):
        n = x.shape[0] // 8
        return jnp.where(never[None], v8[None], x.reshape(n, 8, 128)).reshape(x.shape)

    def gated(v, rel):
        return jnp.concatenate(
            [sel(never_a[0], rel, v[:, g * 128:(g + 1) * 128]) for g in range(v.shape[1] // 128)], axis=1)

    def layernorm(c, rels=None):
        hp = LNP // 2
        for j in range(TK // LNP):
            r0 = c * TK + j * hp
            x = jnp.concatenate([x_s[r0:r0 + hp, :], x_s[r0 + TK // 2:r0 + TK // 2 + hp, :]], axis=0)
            if rels is not None:
                x = _upk(gated(pltpu.bitcast(x, u32), rels[j]))
            x = _up(x)
            mu = jnp.mean(x, axis=-1, keepdims=True)
            xc = x - mu
            var = jnp.mean(xc * xc, axis=-1, keepdims=True)
            if c == 0 and j == 0:
                never_a[0] = jnp.broadcast_to(var[0:8, :], (8, 128)) < -1.0
            xn = xc * lax.rsqrt(var + EPS)
            p0 = c * TK // 2 + j * hp
            lo, hi = xn[0:hp], xn[hp:LNP]
            xn_s[_h2(p0, p0 + hp), :] = _pk(lo)
            xn_s[_h2(SH + p0, SH + p0 + hp), :] = _pk(hi)
            sums = _b_sums(lo[:, 0:256], hi[:, 0:256], lo[:, 256:512], hi[:, 256:512])
            for i in range(5):
                _put(xb_s, (i,), _h2(p0, p0 + hp), _ALL, sums[i])

    def kproj(c):
        lo, hi = _h2(c * TK // 2, (c + 1) * TK // 2), _h2(SH + c * TK // 2, SH + (c + 1) * TK // 2)
        k = _mm(_upk(jnp.concatenate([xn_s[lo, :], xn_s[hi, :]], axis=0)), wqkv_s[:, D:2 * D])
        k_s[lo, :] = _pk(k[0:TK // 2])
        k_s[hi, :] = _pk(k[TK // 2:TK])
        return [_bits(k[j * LNP:j * LNP + 8, 0:128]) for j in range(TK // LNP)]

    def kpost(c, ku):
        rows = _h2(c * TK, (c + 1) * TK)
        for p in range(NPAIR):
            g, lo = divmod(2 * DH * p, 128)
            tile = ku[:, g * 128:(g + 1) * 128]
            if lo + 2 * DH > 128:
                tile = jnp.where(lane_a >= 64, tile, ku[:, (g + 1) * 128:(g + 2) * 128])
            if lo != 8:
                tile = pltpu.roll(tile, (8 - lo) % 128, 1)
            kp_s[p, rows, :] = jnp.where(lane_a < 8, one_lane, tile)

    def knorm(ku):
        kf = _up(_upk(ku))
        kn = _nt(et16, (kf * kf).astype(bf16))
        for j in range(TK // 128):
            kj = kn[:, j * 128:(j + 1) * 128]
            kmax[0] = kj if kmax[0] is None else jnp.maximum(kmax[0], kj)

    def prep_square(i, w):
        t = _up(w).T
        _put(wt_s, (i,), _ALL, _ALL, t)
        sums = _a_sums(t[0:DHALF, 0:256], t[0:DHALF, 256:512], t[DHALF:D, 0:256], t[DHALF:D, 256:512])
        for j in range(5):
            _put(wa_s, (i, j), _ALL, _ALL, sums[j])

    def strassen_x(a, n0, hold=None):
        lo, hi = _h2(n0, n0 + NB), _h2(SH + n0, SH + n0 + NB)
        xe = jnp.concatenate([xn_s[lo, 512:640], xn_s[hi, 512:640]], axis=0)
        if hold is not None:
            xe = _hold(hold[0], hold[1], xe)
        xe = _upk(xe)
        m1 = _nt(a[0], _upk(xb_s[0, lo]))
        m2 = _nt(a[1], _upk(xn_s[lo, 0:256]))
        m3 = _nt(a[2], _upk(xb_s[1, lo]))
        m4 = _nt(a[3], _upk(xb_s[2, lo]))
        m5 = _nt(a[4], _upk(xn_s[hi, 256:512]))
        m6 = _nt(a[5], _upk(xb_s[3, lo]))
        m7 = _nt(a[6], _upk(xb_s[4, lo]))
        e1 = _nt(a[7], xe)
        e2 = _nt(a[8], xe)
        c11, c12, c21, c22 = _combine(m1, m2, m3, m4, m5, m6, m7)
        return c11 + e1[:, 0:NB], c12 + e1[:, NB:], c21 + e2[:, 0:NB], c22 + e2[:, NB:]

    def proj_t(i, n0, r):
        top, bot = _h2(r, r + MQ), _h2(DHALF + r, DHALF + r + MQ)
        a = (_upk(wa_s[i, 0, top]), _upk(wa_s[i, 1, top]), _upk(wt_s[i, top, 0:256]),
             _upk(wt_s[i, bot, 256:512]), _upk(wa_s[i, 2, top]), _upk(wa_s[i, 3, top]),
             _upk(wa_s[i, 4, top]), _upk(wt_s[i, top, 512:640]), _upk(wt_s[i, bot, 512:640]))
        c11, c12, c21, c22 = strassen_x(a, n0)
        lo, hi = slice(n0, n0 + NB), slice(SH + n0, SH + n0 + NB)
        p0 = r // 40
        return ((c11, p0, lo), (c12, p0, hi), (c21, NPAIR // 2 + p0, lo), (c22, NPAIR // 2 + p0, hi))

    def allsum8(v):
        for sh in (4, 2, 1):
            v = v + pltpu.roll(v, sh, 0)
        return v

    def neg_bound(n2, h):
        kr = jnp.concatenate([jnp.broadcast_to(kr_s[pl.ds(h, 1), :], (8, 128))] * (NB // 128), axis=1)
        root = pltpu.bitcast((pltpu.bitcast(n2, jnp.int32) >> 1) + 0x1FC00000, f32)
        return _rnd(root * kr)

    def store_q(qt, p0, cols):
        qt = qt * QSCALE
        z8 = jnp.zeros((8, NB), f32)
        for j in range(MQ // 40):
            p = p0 + j
            t = [qt[40 * j + 8 * i:40 * j + 8 * i + 8, :] for i in range(5)]
            ta, tb = jnp.where(sub_b < 4, t[2], 0.0), jnp.where(sub_b >= 4, t[2], 0.0)
            ma = neg_bound(allsum8(t[0] * t[0] + t[1] * t[1] + ta * ta), 2 * p)
            mb = neg_bound(allsum8(tb * tb + t[3] * t[3] + t[4] * t[4]), 2 * p + 1)
            qt_s[p, :, cols] = jnp.concatenate(t + [ma, mb], axis=0)
            _put(qw_s, (2 * p,), slice(0, 16), cols, jnp.concatenate([ma, t[0], t[1], ta], axis=0))
            _put(qw_s, (2 * p + 1,), _ALL, cols, jnp.concatenate([mb, z8, z8, tb, t[3], t[4]], axis=0))

    def store_v(vt, p0, cols):
        for j in range(MQ // 40):
            b = 40 * j
            mid = vt[b + 16:b + 24, :]
            vt_s[p0 + j, :, cols] = jnp.concatenate(
                [vt[b:b + 16, :], jnp.where(sub_b < 4, mid, 1.0), jnp.where(sub_b >= 4, mid, 1.0),
                 vt[b + 24:b + 40, :]], axis=0)

    x_copy(0).start()
    x_copy(1).start()
    wqkv_copy(1).start()
    x_copy(0).wait()
    layernorm(0)
    x_copy(1).wait()
    wqkv_copy(1).wait()
    x_copy(2).start()
    x_copy(3).start()
    layernorm(1, kproj(0))
    x_copy(2).wait()
    wqkv_copy(2).start()
    wqkv_copy(0).start()
    layernorm(2, kproj(1))
    layernorm(3, kproj(2))
    x_copy(3).wait()
    for c in range(3, 6):
        layernorm(c + 1, kproj(c))
    wqkv_copy(0).wait()
    wqkv_copy(2).wait()
    wg_copy.start()
    wu_copy.start()
    wd_copy.start()
    wo_copy.start()
    prep_square(1, wqkv_s[:, 2 * D:3 * D])
    layernorm(7, kproj(6))
    kproj(7)

    kbs = (kba_s, kbb_s)

    def kb_piece(pair, par, t, d0, d1, pin=None):
        src = kp_s[pair, _h2((t + 1) * KC - NV, (t + 1) * KC), :]
        if pin is not None:
            src = sel(pin[0], pltpu.bitcast(pin[1], u32), src)
        for d in range(d0, d1):
            ln = 8 + DH * par + d
            kbs[par][t, d] = _up(_upk(jnp.broadcast_to(src[:, ln:ln + 1], (NV // 2, 128))))

    blocks = [(n0, r) for n0 in range(0, SH, NB) for r in range(0, DHALF, MQ)]
    nh = len(blocks) // 2
    ku = None
    for b, (n0, r) in enumerate(blocks[:nh]):
        outs = proj_t(1, n0, r)
        if ku is not None:
            knorm(ku)
        if b == 0:
            prep_square(0, wqkv_s[:, 0:D])
        for c in range(b * (S // TK) // nh, (b + 1) * (S // TK) // nh):
            ku = gated(k_s[_h2(c * TK, (c + 1) * TK), :], pltpu.bitcast(outs[0][0][0:8, 0:128], u32))
            kpost(c, ku)
        for o in outs:
            store_v(*o)
    for b, (n0, r) in enumerate(blocks):
        outs = proj_t(0, n0, r)
        if b == 0:
            knorm(ku)
            k2 = jnp.max(kmax[0], axis=1, keepdims=True)
            kr_s[...] = jnp.broadcast_to(jnp.sqrt(k2) * -1.02, (H, 128))
        for o in outs:
            store_q(*o)
    for b, (n0, r) in enumerate(blocks[nh:]):
        if b < nh - 1:
            for t in range(b * NT // (nh - 1), (b + 1) * NT // (nh - 1)):
                for par in range(2):
                    kb_piece(0, par, t, 0, DH, (never_a[0], outs[par][0][0:8, 0:128]))
        outs = proj_t(1, n0, r)
        for o in outs:
            store_v(*o)

    def qk(pair, par, qi, t, never=None):
        kw = 32 if par == 0 else 48
        rs = list(range(KC - NV - 16, -1, -16))
        lhs = jnp.concatenate([kp_s[pair, _h2(t * KC + r0, t * KC + r0 + 16), :] for r0 in rs], axis=0)
        w = qw_s[2 * pair + par, 0:kw // 2, qi * TQ:(qi + 1) * TQ]
        if never is not None:
            late = qt_s[pair, 0:8, 0:128]
            for _ in range(STAGGER):
                late = late * 1.5
            late = pltpu.bitcast(late, u32)
            w = jnp.concatenate(
                [w[:, 0:128], w[:, 128:256], sel(never, late, w[:, 256:384]), sel(never, late, w[:, 384:512])],
                axis=1)
        s = _mm(_upk(lhs)[:, 0:kw], _upk(w))
        e = jnp.exp2(s)
        return s, [e[i * 16:(i + 1) * 16, :] for i in range(len(rs))][::-1]

    def vqk(pair, par, qi, t, never, relv):
        css = [slice(qi * TQ + cc * 128, qi * TQ + (cc + 1) * 128) for cc in range(NCOL)]
        cols = [jnp.concatenate([qt_s[pair, 40 + 8 * par:48 + 8 * par, css[cc]]] * (NV // 8), axis=0)
                for cc in range(NCOL)]
        for d in range(DH):
            kb = kbs[par][t, d]
            if relv is not None and d in GATES:
                r = (GATES.index(d) * (relv.shape[0] // 8)) // len(GATES)
                kb = sel(never, relv[r * 8:(r + 1) * 8, 0:128], kb)
            for cc in range(NCOL):
                cols[cc] = cols[cc] + kb * qt_s[pair, pl.ds(DH * par + d, 1), css[cc]]
        return jnp.exp2(jnp.concatenate(cols, axis=1))

    row8 = lax.broadcasted_iota(jnp.int32, (8, 128), 0)
    slots = [(par, t, qi) for par in range(2) for t in range(NT) for qi in range(NQ)]

    def pv(pair, par, t, qi, p, bad):
        rows, cs = slice(24 * par, 24 * par + 24), slice(qi * TQ, (qi + 1) * TQ)
        acc = _mm(vt_s[pair, rows, t * KC:(t + 1) * KC], p)
        if t > 0:
            acc = acc + ot_s[pair, rows, cs]
        ot_s[pair, rows, cs] = acc
        if t == NT - 1:
            lr = 20 if par == 0 else 0
            l = acc[lr:lr + 1, :]
            bad = jnp.maximum(bad, jnp.where((l >= L_LO) & (l <= L_HI), 0.0, 1.0))
        return bad

    def body(pair, bad):
        never = (row8 + pair) < 0
        nxt = jnp.minimum(pair + 1, NPAIR - 1)
        hist = []
        pend = None
        for i, (par, t, qi) in enumerate(slots):
            ev = vqk(pair, par, qi, t, never, hist[-1]) if hist else ev_s[...]
            if i >= NQ:
                ppar, pt, _ = slots[i - NQ]
                kb_piece(nxt, ppar, pt, qi * 5, qi * 5 + 5, (never, hist[-1][0:8, 0:128]))
            s, parts = qk(pair, par, qi, t, never if i == 0 else None)
            hist.append(s)
            if pend is None:
                bad = pv(jnp.maximum(pair - 1, 0), *slots[-1], pc_s[...], bad)
            else:
                bad = pv(pair, *pend[:3], jnp.concatenate(pend[3], axis=0), bad)
            pend = (par, t, qi, parts + [ev])
        kb_piece(nxt, 1, NT - 1, 0, DH, (never, hist[-3][0:8, 0:128]))
        pc_s[...] = jnp.concatenate(pend[3], axis=0)
        ev_s[...] = vqk(nxt, 0, 0, 0, never, hist[-1])
        return bad

    pc_s[...] = jnp.zeros((KC, TQ), f32)
    ev_s[...] = vqk(0, 0, 0, 0, None, None)
    ot_s[0, 24:48, S - TQ:S] = jnp.ones((24, TQ), f32)
    wg_copy.wait()
    wu_copy.wait()
    wd_copy.wait()
    wo_copy.wait()
    bad = lax.fori_loop(0, NPAIR, body, jnp.zeros((1, TQ), f32))
    bad = pv(NPAIR - 1, *slots[-1], pc_s[...], bad)

    never_c = kr_s[0:8, :] > 1.0
    wd_s[F:F + 64, :] = jnp.zeros((64, D), bf16)
    for i in range(7):
        hb_s[i, _h2(FH, FP), :] = jnp.zeros(((FP - FH) // 2, SH), u32)

    def strip_t(w_s, r0, rel):
        v = pltpu.bitcast(w_s[r0:r0 + 128, :], u32)
        relu = pltpu.bitcast(rel, u32)
        v = jnp.concatenate([sel(never_c, relu, v[:, j * 128:(j + 1) * 128]) for j in range(D // 128)], axis=1)
        return _up(_upk(v)).T

    def prep_piece(i, rel):
        if i < FP // 128:
            cs = slice(i * 128, (i + 1) * 128)
            t0, t1 = strip_t(wd_s, i * 128, rel), strip_t(wd_s, FH + i * 128, rel)
            vals = _a_sums(t0[0:DHALF], t1[0:DHALF], t0[DHALF:D], t1[DHALF:D])
            _put(wdt_s, (0,), _ALL, cs, t0[0:DHALF])
            _put(wdt_s, (1,), _ALL, cs, t1[DHALF:D])
            for j in range(5):
                _put(wda_s, (j,), _ALL, cs, vals[j])
            vals = vals[1:3]
        elif i < FP // 128 + 2:
            i -= FP // 128
            cs = slice(i * 128, (i + 1) * 128)
            t0, t1 = strip_t(wo_s, i * 128, rel), strip_t(wo_s, 256 + i * 128, rel)
            vals = _a_sums(t0[0:DHALF], t1[0:DHALF], t0[DHALF:D], t1[DHALF:D])
            _put(wt_s, (2,), _ALL, cs, t0)
            _put(wt_s, (2,), _ALL, slice(256 + i * 128, 256 + (i + 1) * 128), t1)
            for j in range(5):
                _put(wa_s, (2, j), _ALL, cs, vals[j])
            vals = vals[1:3]
        else:
            vals = [strip_t(wo_s, 512, rel)]
            _put(wt_s, (2,), _ALL, slice(512, 640), vals[0])
        return never_c, _or_tiles([_bits(v) for v in vals])

    def ffn_a(w_s, r):
        r1, r2 = slice(r, r + MF), slice(FH + r, FH + r + MF)
        a11, a12, a21, a22 = w_s[r1, 0:256], w_s[r1, 256:512], w_s[r2, 0:256], w_s[r2, 256:512]
        s1, s2, s5, s6, s7 = [v.astype(bf16) for v in _a_sums(_up(a11), _up(a12), _up(a21), _up(a22))]
        return s1, s2, a11, a22, s5, s6, s7, w_s[r1, 512:640], w_s[r2, 512:640]

    blk = 0
    holds = {}
    for j in range(FH // MF):
        r = j * MF
        ag, au = ffn_a(wg_s, r), ffn_a(wu_s, r)
        for n0 in range(0, SH, NB):
            g = strassen_x(ag, n0, holds.pop(blk, None))
            u = strassen_x(au, n0)
            h11, h12, h21, h22 = [_silu(a) * b for a, b in zip(g, u)]
            t1_, t3, t4, t6, t7 = _b_sums(h11, h12, h21, h22)
            for i, v in enumerate((t1_, h11, t3, t4, h22, t6, t7)):
                _put(hb_s, (i,), _h2(r, r + MF), slice(n0, n0 + NB), v)
            if blk in PREPAT:
                holds[blk + 2] = prep_piece(PREPAT.index(blk), t7[MF - 8:MF, NB - 128:NB])
            blk += 1

    def out_copy(i):
        return pltpu.make_async_copy(
            out_s.at[pl.ds(i * 128, 128), :], out_hbm.at[0, pl.ds(i * 128, 128), :], sem.at[0])

    def final_block(c0, tn, start_copies, tok=None):
        def ds(a, n):
            return slice(a, a + n) if isinstance(a, int) else pl.ds(pl.multiple_of(a, 128), n)

        sub_n = lax.broadcasted_iota(jnp.int32, (8, tn), 0)

        def o_tile(cs):
            parts = []
            for p in range(NPAIR):
                ra = 1.0 / ot_s[p, 20:21, cs]
                rb = 1.0 / ot_s[p, 24:25, cs]
                parts.append(ot_s[p, 0:16, cs] * ra)
                parts.append(jnp.where(sub_n < 4, ot_s[p, 16:24, cs] * ra, ot_s[p, 24:32, cs] * rb))
                parts.append(ot_s[p, 32:48, cs] * rb)
            return jnp.concatenate(parts, axis=0)

        top, bot = _h2(0, DHALF), _h2(DHALF, D)
        olo, ohi = o_tile(ds(c0, tn)), o_tile(ds(SH + c0, tn))
        b11, b21, b12, b22 = olo[0:256], olo[256:512], ohi[0:256], ohi[256:512]
        t1_, t3, t4, t6, t7 = _b_sums(b11, b12, b21, b22)
        lhs = (wa_s[2, 0], wa_s[2, 1], wt_s[2, top, 0:256], wt_s[2, bot, 256:512],
               wa_s[2, 2], wa_s[2, 3], wa_s[2, 4])
        s11, s12, s21, s22 = _combine(*[
            _mm(_upk(a), b.astype(bf16)) for a, b in zip(lhs, (t1_, b11, t3, t4, b22, t6, t7))])
        e = _mm(_upk(wt_s[2, :, 512:640]),
                jnp.concatenate([olo[512:640], ohi[512:640]], axis=1).astype(bf16))
        lhs = (wda_s[0], wda_s[1], wdt_s[0], wdt_s[1], wda_s[2], wda_s[3], wda_s[4])
        rhs = [hb_s[i, :, ds(c0, tn)] for i in range(7)]
        if tok is not None:
            rhs[3] = _hold(never_c, tok, rhs[3])
        f11, f12, f21, f22 = _combine(*[_mm(_upk(a), _upk(b)) for a, b in zip(lhs, rhs)])
        ys = (((jnp.concatenate([s11, s21], axis=0) + e[:, 0:tn])
               * _silu(jnp.concatenate([f11, f21], axis=0))).T,
              ((jnp.concatenate([s12, s22], axis=0) + e[:, tn:])
               * _silu(jnp.concatenate([f12, f22], axis=0))).T)
        done = []
        for j in range(tn // 128):
            for half in range(2):
                r0 = 2 * c0 + (2 * j + half) * 128
                rows = ds(r0, 128)
                o = _up(x_s[rows, :]) + ys[half][j * 128:(j + 1) * 128]
                out_s[rows, :] = o.astype(bf16)
                if start_copies:
                    out_copy(r0 // 128).start()
                done.append(_bits(o))
        return _or_tiles(done) if start_copies else None

    c0 = 0
    tok = None
    for tn in TNS:
        tok = final_block(c0, tn, True, tok)
        c0 += tn

    @pl.when(jnp.max(bad) > 0.0)
    def _():
        for i in range(S // 128):
            out_copy(i).wait()
        row_q = lax.broadcasted_iota(jnp.int32, (40, TQ), 0)

        def fb(j, carry):
            pair = j // NQ
            cols = pl.ds(pl.multiple_of((j % NQ) * TQ, TQ), TQ)
            for par in range(2):
                mine = (row_q < DH) if par == 0 else (row_q >= DH)
                qm = jnp.concatenate(
                    [jnp.zeros((8, TQ), f32), jnp.where(mine, qt_s[pair, 0:40, cols], 0.0)], axis=0)
                sc_s[...] = _mm(_upk(kp_s[pair])[:, 0:48], qm.astype(bf16))
                m = jnp.max(sc_s[...], axis=0, keepdims=True)
                p = jnp.exp2(sc_s[...] - m)
                ot_s[pair, 24 * par:24 * par + 24, cols] = _mm(vt_s[pair, 24 * par:24 * par + 24, :], p)
            return carry
        lax.fori_loop(0, NPAIR * NQ, fb, 0)

        def redo(c, carry):
            final_block(c * 128, 128, False)
            return carry
        lax.fori_loop(0, SH // 128, redo, 0)
        for i in range(S // 128):
            out_copy(i).start()

    for i in range(S // 128):
        out_copy(i).wait()


@jax.jit
def pallas_recurrent_scan__mha_block__swiglu_ffn__prompt_kernel(
    A_x: jax.Array,
    A_wqkv: jax.Array,
    A_wo: jax.Array,
    B_x: jax.Array,
    B_w_gate: jax.Array,
    B_w_up: jax.Array,
    B_w_down: jax.Array,
):
    del B_x
    hbm = pl.BlockSpec(memory_space=pltpu.HBM)
    return pl.pallas_call(
        _kernel,
        out_shape=jax.ShapeDtypeStruct((1, S, D), bf16),
        in_specs=[hbm] * 6,
        out_specs=hbm,
        scratch_shapes=[
            pltpu.VMEM((S, D), bf16),
            pltpu.VMEM((D, 3 * D), bf16),
            pltpu.VMEM((D, D), bf16),
            pltpu.VMEM((F, D), bf16),
            pltpu.VMEM((F, D), bf16),
            pltpu.VMEM((F + 64, D), bf16),
            pltpu.VMEM((S // 2, D), u32),
            pltpu.VMEM((5, SH // 2, 256), u32),
            pltpu.VMEM((3, D // 2, D), u32),
            pltpu.VMEM((3, 5, DHALF // 2, 256), u32),
            pltpu.VMEM((S // 2, D), u32),
            pltpu.VMEM((NPAIR, S // 2, 128), u32),
            pltpu.VMEM((NPAIR, 56, S), f32),
            pltpu.VMEM((H, 24, S), u32),
            pltpu.VMEM((NPAIR, 48, S), f32),
            pltpu.VMEM((H, 128), f32),
            pltpu.VMEM((NT, DH, NV, 128), f32),
            pltpu.VMEM((NT, DH, NV, 128), f32),
            pltpu.VMEM((NPAIR, 48, S), f32),
            pltpu.VMEM((7, FP // 2, SH), u32),
            pltpu.VMEM((2, DHALF // 2, FP), u32),
            pltpu.VMEM((5, DHALF // 2, FP), u32),
            pltpu.VMEM((S, D), bf16),
            pltpu.VMEM((S, TQ), f32),
            pltpu.VMEM((KC, TQ), f32),
            pltpu.VMEM((NV, TQ), f32),
            pltpu.SemaphoreType.DMA((4,)),
        ],
        compiler_params=pltpu.CompilerParams(vmem_limit_bytes=120 * 1024 * 1024),
    )(A_x, A_wqkv, A_wo, B_w_gate.T, B_w_up.T, B_w_down)
```
